```python
import jax
import jax.numpy as jnp

def _softmax(x, axis=-1):
    return jax.nn.softmax(x, axis=axis)

def _gelu(x):
    return jax.nn.gelu(x, approximate=True)

def _silu(x):
    return jax.nn.silu(x)

def _sigmoid(x):
    return jax.nn.sigmoid(x)

def _layernorm(x, axis=-1, eps=1e-05):
    m = jnp.mean(x, axis=axis, keepdims=True)
    v = jnp.var(x, axis=axis, keepdims=True)
    return (x - m) / jnp.sqrt(v + eps)

def _scatter_add(tgt, idx, src, axis=0):
    return tgt.at[idx].add(src)

def _segment_sum(src, seg, n):
    return jax.ops.segment_sum(src, seg, n)

class _Rng:

    def __init__(self, key):
        self._k = key

    def _next(self):
        self._k, sub = jax.random.split(self._k)
        return sub

    def normal(self, shape):
        return jax.random.normal(self._next(), shape, dtype=jnp.bfloat16)

    def randint(self, lo, hi, shape):
        return jax.random.randint(self._next(), shape, lo, hi, dtype=jnp.int32)

    def uniform(self, shape, lo=0.0, hi=1.0):
        return jax.random.uniform(self._next(), shape, jnp.bfloat16, lo, hi)

    def permutation(self, n):
        return jax.random.permutation(self._next(), n)
kernel_name = 'adaLN_cond__ssm_conv_h3__glu_gated_reglu__prompt'

def setup_inputs():
    _rng = _Rng(jax.random.key(int.from_bytes(__import__("os").urandom(4), "little")))
    _w = lambda a: (lambda t: t.astype(jnp.bfloat16) if jnp.issubdtype(t.dtype, jnp.floating) else t)(jnp.asarray(a))

    def _A_setup():
        B, S, D = (1, 2048, 640)
        ks = 4
        return {'q': _w((lambda *s: _rng.normal(s) * 0.05)(B, S, D)), 'k': _w((lambda *s: _rng.normal(s) * 0.05)(B, S, D)), 'v': _w((lambda *s: _rng.normal(s) * 0.05)(B, S, D)), 'shift_k': _w((lambda *s: _rng.normal(s) * 0.05)(D, ks) * 0.5), 'ssm_k': _w((lambda *s: _rng.normal(s) * 0.05)(D, S) * (1.0 / S ** 0.5)), 'ssm_D': _w((lambda *s: _rng.normal(s) * 0.05)(D))}
    _A_in = _A_setup()

    def _B_setup():
        B, S, D, F = (1, 2048, 640, 1536)
        return {'x': _w((lambda *s: _rng.normal(s) * 0.05)(B, S, D)), 'W_gate': _w((lambda *s: _rng.normal(s) * 0.05)(D, F) * (2.0 / D) ** 0.5), 'W_up': _w((lambda *s: _rng.normal(s) * 0.05)(D, F) * (2.0 / D) ** 0.5), 'W_down': _w((lambda *s: _rng.normal(s) * 0.05)(F, D) * (1.0 / F) ** 0.5)}
    _B_in = _B_setup()
    return {'A_q': _A_in['q'], 'A_k': _A_in['k'], 'A_v': _A_in['v'], 'A_shift_k': _A_in['shift_k'], 'A_ssm_k': _A_in['ssm_k'], 'A_ssm_D': _A_in['ssm_D'], 'B_x': _B_in['x'], 'B_W_gate': _B_in['W_gate'], 'B_W_up': _B_in['W_up'], 'B_W_down': _B_in['W_down'], 'c': _w((lambda *s: _rng.normal(s) * 0.05)(1, 640)), 'w_mod': _w((lambda *s: _rng.normal(s) * 0.05)(640, 6 * 640) * 640 ** (-0.5))}

def reference(A_q, A_k, A_v, A_shift_k, A_ssm_k, A_ssm_D, B_x, B_W_gate, B_W_up, B_W_down, c, w_mod):

    def _A_ref(q, k, v, shift_k, ssm_k, ssm_D):
        B, S, D = q.shape
        ks = shift_k.shape[-1]
        k_pad = jnp.pad(k, ((0, 0), (ks - 1, 0), (0, 0)))
        k_shift = jnp.zeros_like(k)
        for t in range(ks):
            k_shift = k_shift + k_pad[:, t:t + S, :] * shift_k[:, ks - 1 - t][None, None, :]
        kv = k_shift * v
        L = 2 * S
        kv_pad = jnp.pad(kv, ((0, 0), (0, S), (0, 0)))
        kf_pad = jnp.pad(ssm_k, ((0, 0), (0, S)))
        kv_f = (lambda x, axes=(-2, -1): jnp.fft.rfft2(x.astype(jnp.float32), axes=axes))(kv_pad[:, None, :, :], axes=(1, 2))
        kf_f = (lambda x, axes=(-2, -1): jnp.fft.rfft2(x.astype(jnp.float32), axes=axes))(kf_pad[:, None, :], axes=(1, 2))
        kf_f = (lambda x, *d: x.transpose(*d))(kf_f, 1, 2, 0)
        y_f = kv_f * kf_f[None, :, :, :]
        y = (lambda x, s, axes=(-2, -1): jnp.fft.irfft2(x, s=s, axes=axes).astype(jnp.bfloat16))(y_f, (1, L), axes=(1, 2))[:, 0, :S, :]
        y = y + kv * ssm_D[None, None, :]
        return q * y

    def _B_ref(x, W_gate, W_up, W_down):
        gate = jnp.einsum('bsd,df->bsf', x, W_gate)
        up = jnp.einsum('bsd,df->bsf', x, W_up)
        gate = gate * (lambda x, dt: x.astype(dt))(gate > 0, gate.dtype)
        h = gate * up
        return jnp.einsum('bsf,fd->bsd', h, W_down)
    x = A_q
    mod = (_silu(c) @ w_mod).reshape(c.shape[0], 6, 1, -1)
    sa, ca, ga, sb, cb, gb = (mod[:, 0].copy(), mod[:, 1].copy(), mod[:, 2].copy(), mod[:, 3].copy(), mod[:, 4].copy(), mod[:, 5].copy())
    h = _layernorm(x, axis=-1) * (1 + ca) + sa
    x = x + ga * _A_ref(h, A_k, A_v, A_shift_k, A_ssm_k, A_ssm_D)
    h = _layernorm(x, axis=-1) * (1 + cb) + sb
    x = x + gb * _B_ref(h, B_W_gate, B_W_up, B_W_down)
    return x
```

```python
import functools

import numpy as np
import jax
import jax.numpy as jnp
import jax.experimental.pallas as pl
import jax.experimental.pallas.tpu as pltpu

S, D, F = 2048, 640, 1536
C = 128
NCH = S // C
NLT = D // 128
NCOL = 16 * NLT
M = 256
NB = S // M
EPS = 1e-5


def _dft_consts():
    n = 2 * C
    f = np.arange(C)
    t = np.arange(C)
    th = 2 * np.pi * (f[:, None] + 0.5) * t[None, :] / n
    p = 1j * (-1.0) ** f
    fwd, inv = [], []
    for q in range(4):
        a = (p ** (-q))[:, None] * np.exp(-1j * th)
        fwd.append(np.stack([a.real.reshape(16, 8, C), a.imag.reshape(16, 8, C)], 1).reshape(2 * C, C))
        e = (p ** q)[:, None] * np.exp(1j * th)
        g = np.stack([e.real.reshape(16, 8, C), -e.imag.reshape(16, 8, C)], 1).reshape(2 * C, C)
        inv.append((2.0 / n) * g.T)
    return np.stack(fwd).astype(np.float32), np.stack(inv).astype(np.float32)


_FWD_NP, _INV_NP = _dft_consts()


def _ln(x):
    mu = jnp.sum(x, axis=-1, keepdims=True) * (1.0 / D)
    xc = x - mu
    var = jnp.sum(xc * xc, axis=-1, keepdims=True) * (1.0 / D)
    return xc * jax.lax.rsqrt(var + EPS)


def _kernel(x_hbm, k_hbm, v_hbm, sk_hbm, ssmk_hbm, ssmd_hbm, wg_hbm, wu_hbm, wd_hbm, c_hbm, wmod_hbm,
            fwd_hbm, inv_hbm, o_hbm,
            x_v, k_v, v_v, kv_v, sk_v, ssmk_v, ssmd_v, wg_v, wu_v, wd_v, c_v, wmod_v, fwd_v, inv_v,
            X_v, H_v, W_v, mod_v, h2_v, x1_v, act_v, o_v, sems, osem):
    G = 4
    GR = G * C
    copies = {}
    order = []

    def add(name, src, dst):
        cp = pltpu.make_async_copy(src, dst, sems.at[len(order)])
        copies[name] = cp
        order.append(cp)

    add("c", c_hbm, c_v)
    add("sk", sk_hbm, sk_v)
    add("ssmd", ssmd_hbm, ssmd_v)
    add("fwd", fwd_hbm, fwd_v)
    for g in range(NCH // G):
        add(f"k{g}", k_hbm.at[pl.ds(g * GR, GR)], k_v.at[pl.ds(16 + g * GR, GR)])
        add(f"v{g}", v_hbm.at[pl.ds(g * GR, GR)], v_v.at[pl.ds(g * GR, GR)])
        add(f"s{g}", ssmk_hbm.at[:, pl.ds(g * GR, GR)], ssmk_v.at[g])
        if g == 0:
            add("inv", inv_hbm, inv_v)
    for t in range(NLT):
        add(f"wm{t}", wmod_hbm.at[pl.ds(t * 128, 128)], wmod_v.at[pl.ds(t * 128, 128)])
    add("x0", x_hbm.at[pl.ds(0, M)], x_v.at[pl.ds(0, M)])
    add("wg", wg_hbm, wg_v)
    add("wu", wu_hbm, wu_v)
    add("wd", wd_hbm, wd_v)
    add("x1", x_hbm.at[pl.ds(M, S - M)], x_v.at[pl.ds(M, S - M)])
    for cp in order:
        cp.start()

    def wait(*names):
        for nm in names:
            copies[nm].wait()

    k_v[0:16, :] = jnp.zeros((16, D), jnp.bfloat16)
    wait("sk", "fwd")
    taps = jnp.transpose(sk_v[...].astype(jnp.float32))
    w = [taps[j:j + 1, :] for j in range(4)]

    def spectrum_parts(spec, col):
        lt, fg = divmod(col, 16)
        re = spec[16 * fg:16 * fg + 8, 128 * lt:128 * lt + 128]
        im = spec[16 * fg + 8:16 * fg + 16, 128 * lt:128 * lt + 128]
        return re, im

    def fwd_group(g):
        for q in range(G):
            i = g * G + q
            r0 = i * C
            kf = k_v[r0:r0 + C + 16, :].astype(jnp.float32)
            ks = w[0] * kf[16:16 + C]
            for j in range(1, 4):
                ks = ks + w[j] * kf[16 - j:16 - j + C]
            kv = (ks * v_v[r0:r0 + C, :].astype(jnp.float32)).astype(jnp.bfloat16)
            kv_v[r0:r0 + C, :] = kv
            xs = jnp.dot(fwd_v[q], kv, preferred_element_type=jnp.float32)
            hs = jax.lax.dot_general(fwd_v[q], ssmk_v[g, :, q * C:(q + 1) * C],
                                     (((1,), (1,)), ((), ())), preferred_element_type=jnp.float32)
            for col in range(NCOL):
                re, im = spectrum_parts(xs, col)
                X_v[i, col, 0:8, :] = re + im
                X_v[i, col, 8:16, :] = re
                X_v[i, col, 16:24, :] = im
                re, im = spectrum_parts(hs, col)
                H_v[i, col, 0:8, :] = re
                H_v[i, col, 8:16, :] = im - re
                H_v[i, col, 16:24, :] = im + re

    for g in range(NCH // G):
        wait(f"k{g}", f"v{g}", f"s{g}")
        fwd_group(g)

    wait("c")
    cf = c_v[...].astype(jnp.float32)
    sc = (cf * jax.nn.sigmoid(cf)).astype(jnp.bfloat16)
    sc = jnp.broadcast_to(sc, (16, D))
    acc = None
    for t in range(NLT):
        wait(f"wm{t}")
        part = jnp.dot(sc[:, t * 128:(t + 1) * 128], wmod_v[t * 128:(t + 1) * 128, :],
                       preferred_element_type=jnp.float32)
        acc = part if acc is None else acc + part
    mod_v[...] = acc[0:8, :]

    BLK = 4

    def prod_col(col, _):
        def ld(ref, j):
            v = ref[j, col]
            return v[0:8], v[8:16], v[16:24]
        zp = None
        for i0 in range(0, NCH, BLK):
            outs = list(range(i0, i0 + BLK))
            acc = {i: None for i in outs}
            hc = {}
            for j in range(outs[-1] + 1):
                xs, xr, xi = ld(X_v, j)
                for i in outs:
                    if i < j:
                        continue
                    m = i - j
                    if m not in hc:
                        hc[m] = ld(H_v, m)
                    hr, hd, hs = hc[m]
                    t = (hr * xs, hd * xr, hs * xi)
                    acc[i] = t if acc[i] is None else tuple(a + b for a, b in zip(acc[i], t))
                for m in list(hc):
                    if m >= outs[-1] - j:
                        del hc[m]
            for i in outs:
                a1, a2, a3 = acc[i]
                zr, zi = a1 - a3, a1 + a2
                wr, wi = (zr, zi) if zp is None else (zr + zp[0], zi + zp[1])
                zp = (zr, zi)
                W_v[i, col] = jnp.concatenate([wr, wi], axis=0).astype(jnp.bfloat16)
        return 0

    jax.lax.fori_loop(0, NCOL, prod_col, 0)

    wait("inv", "ssmd", "x0", "wg", "wu", "wd", "x1")
    mod = mod_v[0:1, :]
    sa, ca, ga, sb, cb, gb = [mod[:, j * D:(j + 1) * D] for j in range(6)]
    dsk = ssmd_v[...].astype(jnp.float32)

    def block(b, _):
        for hq in range(M // C):
            i = b * (M // C) + hq
            r0 = pl.multiple_of(i * C, C)
            gm = inv_v[i % 4]
            ys = []
            for lt in range(NLT):
                wsp = W_v[i, lt * 16:(lt + 1) * 16].reshape(2 * C, 128)
                ys.append(jnp.dot(gm, wsp, preferred_element_type=jnp.float32))
            y = jnp.concatenate(ys, axis=1)
            xf = x_v[pl.ds(r0, C), :].astype(jnp.float32)
            hh = _ln(xf) * (1.0 + ca) + sa
            y = y + kv_v[pl.ds(r0, C), :].astype(jnp.float32) * dsk
            x1 = xf + ga * (hh * y)
            x1_v[hq * C:(hq + 1) * C, :] = x1
            h2_v[hq * C:(hq + 1) * C, :] = (_ln(x1) * (1.0 + cb) + sb).astype(jnp.bfloat16)
        h2 = h2_v[...]
        TN = 512
        for nt in range(F // TN):
            gt = jnp.dot(h2, wg_v[:, nt * TN:(nt + 1) * TN], preferred_element_type=jnp.float32)
            up = jnp.dot(h2, wu_v[:, nt * TN:(nt + 1) * TN], preferred_element_type=jnp.float32)
            act_v[:, nt * TN:(nt + 1) * TN] = (jnp.maximum(gt, 0.0) * up).astype(jnp.bfloat16)
        dn = jnp.dot(act_v[...], wd_v[...], preferred_element_type=jnp.float32)
        rb = pl.multiple_of(b * M, M)
        o_v[pl.ds(rb, M), :] = (x1_v[...] + gb * dn).astype(jnp.bfloat16)
        pltpu.make_async_copy(o_v.at[pl.ds(rb, M)], o_hbm.at[pl.ds(rb, M)], osem).start()
        return 0

    jax.lax.fori_loop(0, NB, block, 0)
    pltpu.make_async_copy(o_v, o_hbm, osem).wait()


@jax.jit
def pallas_adaLN_cond__ssm_conv_h3__glu_gated_reglu__prompt_kernel(
    A_q: jax.Array,
    A_k: jax.Array,
    A_v: jax.Array,
    A_shift_k: jax.Array,
    A_ssm_k: jax.Array,
    A_ssm_D: jax.Array,
    B_x: jax.Array,
    B_W_gate: jax.Array,
    B_W_up: jax.Array,
    B_W_down: jax.Array,
    c: jax.Array,
    w_mod: jax.Array,
):
    del B_x
    bf = jnp.bfloat16
    hbm = pl.BlockSpec(memory_space=pl.ANY)
    scratch = [
        pltpu.VMEM((S, D), bf),
        pltpu.VMEM((S + 16, D), bf),
        pltpu.VMEM((S, D), bf),
        pltpu.VMEM((S, D), bf),
        pltpu.VMEM((D, 4), bf),
        pltpu.VMEM((4, D, 512), bf),
        pltpu.VMEM((1, D), bf),
        pltpu.VMEM((D, F), bf),
        pltpu.VMEM((D, F), bf),
        pltpu.VMEM((F, D), bf),
        pltpu.VMEM((1, D), bf),
        pltpu.VMEM((D, 6 * D), bf),
        pltpu.VMEM((4, 2 * C, C), bf),
        pltpu.VMEM((4, C, 2 * C), bf),
        pltpu.VMEM((NCH, NCOL, 24, 128), jnp.float32),
        pltpu.VMEM((NCH, NCOL, 24, 128), jnp.float32),
        pltpu.VMEM((NCH, NCOL, 16, 128), bf),
        pltpu.VMEM((8, 6 * D), jnp.float32),
        pltpu.VMEM((M, D), bf),
        pltpu.VMEM((M, D), jnp.float32),
        pltpu.VMEM((M, F), bf),
        pltpu.VMEM((S, D), bf),
        pltpu.SemaphoreType.DMA((40,)),
        pltpu.SemaphoreType.DMA(()),
    ]
    out = pl.pallas_call(
        _kernel,
        out_shape=jax.ShapeDtypeStruct((S, D), bf),
        in_specs=[hbm] * 13,
        out_specs=hbm,
        scratch_shapes=scratch,
        compiler_params=pltpu.CompilerParams(vmem_limit_bytes=110 * 1024 * 1024),
    )(
        A_q.reshape(S, D), A_k.reshape(S, D), A_v.reshape(S, D), A_shift_k, A_ssm_k,
        A_ssm_D.reshape(1, D), B_W_gate, B_W_up, B_W_down, c, w_mod,
        jnp.asarray(_FWD_NP, dtype=bf), jnp.asarray(_INV_NP, dtype=bf),
    )
    return out.reshape(1, S, D)
```

```python
import functools

import numpy as np
import jax
import jax.numpy as jnp
import jax.experimental.pallas as pl
import jax.experimental.pallas.tpu as pltpu

S, D, F = 2048, 640, 1536
C = 128
NCH = S // C
NLT = D // 128
NCOL = 16 * NLT
M = 256
NB = S // M
EPS = 1e-5
GS = 32
XB = 0
HB = NCH * NCOL * 16
WB = 2 * HB
ZB = WB + NCH * NCOL * 8
AROWS = ZB + NCH * NCOL * 16

CFG = dict(CHAIN0=False, WD_SPLIT=((0, 384), (384, 640)), UNR_A=2, SR=32, TN=256, G=2, NA=8, BLK_A=8, SCOPES=False,
           FFN_PROD=((0, 1, 8, 14, 20, 0, 1, 'serial'), (1, 4, 8, 14, 20, 20, 1, 'serial'), (4, 7, 14, 16, 27, 0, 1, 'serial'), (7, 8, 0, 0, 0, 0, 1, 'serial')))


def _dft_consts():
    n = 2 * C
    f = np.arange(C)
    t = np.arange(C)
    th = 2 * np.pi * (f[:, None] + 0.5) * t[None, :] / n
    a = np.exp(-1j * th)
    fwd = np.stack([a.real.reshape(16, 8, C), a.imag.reshape(16, 8, C)], 1).reshape(2 * C, C)
    e = np.exp(1j * th)
    g = np.stack([e.real.reshape(16, 8, C), -e.imag.reshape(16, 8, C)], 1).reshape(2 * C, C)
    return fwd.astype(np.float32), ((2.0 / n) * g.T).astype(np.float32)


_FWD_NP, _INV_NP = _dft_consts()


def _ln(x):
    mu = jnp.sum(x, axis=-1, keepdims=True) * (1.0 / D)
    xc = x - mu
    var = jnp.sum(xc * xc, axis=-1, keepdims=True) * (1.0 / D)
    return xc * jax.lax.rsqrt(var + EPS)


class _NoScope:
    def __enter__(self):
        return None

    def __exit__(self, *a):
        return False


def _kernel(x_hbm, k_hbm, v_hbm, sk_hbm, ssmk_hbm, ssmd_hbm, wg_hbm, wu_hbm, wd_hbm, c_hbm, wmod_hbm,
            fwd_hbm, inv_hbm, z_hbm, o_hbm,
            x_v, k_v, v_v, sk_v, ssmk_v, ssmd_v, wg_v, wu_v, wd_v, c_v, wmod_v, fwd_v, inv_v,
            A_v, mod_v, y_v, act_v, o_v, z_s, sems, osem, *, cfg):
    scope = (lambda n: jax.named_scope(n)) if cfg["SCOPES"] else (lambda n: _NoScope())
    SR, TN = cfg["SR"], cfg["TN"]
    G = cfg["G"]
    GR = G * C
    NG = NCH // G
    copies = {}
    order = []

    def add(name, src, dst):
        cp = pltpu.make_async_copy(src, dst, sems.at[len(order)])
        copies[name] = cp
        order.append(cp)

    def group_copies(g):
        r = g * GR
        if not isinstance(g, int):
            r = pl.multiple_of(r, GR)
        return (pltpu.make_async_copy(k_hbm.at[pl.ds(r, GR)], k_v.at[pl.ds(16 + r, GR)], sems.at[GS + 3 * g]),
                pltpu.make_async_copy(v_hbm.at[pl.ds(r, GR)], v_v.at[pl.ds(r, GR)], sems.at[GS + 3 * g + 1]),
                pltpu.make_async_copy(ssmk_hbm.at[:, pl.ds(r, GR)], ssmk_v.at[g], sems.at[GS + 3 * g + 2]))

    add("sk", sk_hbm, sk_v)
    add("ssmd", ssmd_hbm, ssmd_v)
    add("fwd", fwd_hbm, fwd_v.at[0])
    for cp in order:
        cp.start()
    for g in range(NG):
        for cp in group_copies(g):
            cp.start()
    n0 = len(order)
    add("z", z_hbm, z_s)
    add("c", c_hbm, c_v)
    for t in range(NLT):
        add(f"wm{t}", wmod_hbm.at[pl.ds(t * 128, 128)], wmod_v.at[pl.ds(t * 128, 128)])
    add("inv", inv_hbm, inv_v)
    add("x0", x_hbm.at[pl.ds(0, M)], x_v.at[pl.ds(0, M)])
    for nt in range(F // TN):
        add(f"wg{nt}", wg_hbm.at[:, pl.ds(nt * TN, TN)], wg_v.at[:, pl.ds(nt * TN, TN)])
        add(f"wu{nt}", wu_hbm.at[:, pl.ds(nt * TN, TN)], wu_v.at[:, pl.ds(nt * TN, TN)])
    add("x1", x_hbm.at[pl.ds(M, M)], x_v.at[pl.ds(M, M)])
    for (c0, c1) in cfg["WD_SPLIT"]:
        add(f"wd{c0}", wd_hbm.at[:, pl.ds(c0, c1 - c0)], wd_v.at[:, pl.ds(c0, c1 - c0)])
    add("x2", x_hbm.at[pl.ds(2 * M, S - 2 * M)], x_v.at[pl.ds(2 * M, S - 2 * M)])
    for cp in order[n0:]:
        cp.start()

    def wait(*names):
        for nm in names:
            copies[nm].wait()

    k_v[0:16, :] = jnp.zeros((16, D), jnp.bfloat16)
    wait("sk", "fwd", "ssmd")
    taps = sk_v[...].astype(jnp.float32)
    sgn = (1 - 2 * (jax.lax.broadcasted_iota(jnp.int32, (8, 128), 0) % 2)).astype(jnp.float32)
    f0 = fwd_v[0].astype(jnp.float32)
    f1 = []
    for fg in range(16):
        f1.append(sgn * f0[16 * fg + 8:16 * fg + 16])
        f1.append(-sgn * f0[16 * fg:16 * fg + 8])
    f1 = jnp.concatenate(f1, axis=0)
    fwd_v[1] = f1.astype(jnp.bfloat16)
    fwd_v[2] = (-f0).astype(jnp.bfloat16)
    fwd_v[3] = (-f1).astype(jnp.bfloat16)
    w = [taps[j:j + 1, :] for j in range(4)]

    def fwd_group(g):
        for q in range(G):
            i = g * G + q
            r0 = pl.multiple_of(i * C, C)
            fm = fwd_v[i % 4]
            kf = k_v[pl.ds(r0, C + 16), :].astype(jnp.float32)
            ks = w[0] * kf[16:16 + C]
            for j in range(1, 4):
                ks = ks + w[j] * kf[16 - j:16 - j + C]
            kv = (ks * v_v[pl.ds(r0, C), :].astype(jnp.float32)).astype(jnp.bfloat16)
            xs = jnp.dot(fm, kv, preferred_element_type=jnp.float32)
            hs = jax.lax.dot_general(fm, ssmk_v[g, :, q * C:(q + 1) * C],
                                     (((1,), (1,)), ((), ())), preferred_element_type=jnp.float32)
            base = pl.multiple_of(i * (NCOL * 16), 8)
            for col in range(NCOL):
                lt, fg = divmod(col, 16)
                A_v[pl.ds(base + XB + col * 16, 16), :] = xs[16 * fg:16 * fg + 16, 128 * lt:128 * lt + 128]
                A_v[pl.ds(base + HB + col * 16, 16), :] = hs[16 * fg:16 * fg + 16, 128 * lt:128 * lt + 128]

    def add_skip():
        dsk = ssmd_v[...].astype(jnp.float32)
        for col in range(NCOL):
            lt = col // 16
            r = HB + col * 16
            A_v[r:r + 8, :] = A_v[r:r + 8, :] + jnp.broadcast_to(dsk[lt:lt + 1, :], (8, 128))

    def prod_col(col, lo, hi, blk, mode, zs=0):
        def ld(base, j):
            v = A_v[pl.ds(pl.multiple_of(base + (j * NCOL + col) * 16, 8), 16), :]
            return v[0:8], v[8:16]
        zp = None
        if lo > 0:
            zz = A_v[pl.ds(pl.multiple_of(ZB + (lo * NCOL + col) * 16, 8), 16), :]
            zp = (zz[0:8], zz[8:16])
        for i0 in range(lo, hi, blk):
            outs = list(range(i0, min(i0 + blk, hi)))
            acc = {i: None for i in outs}
            hc = {}
            for j in range(outs[-1] + 1):
                xr, xi = ld(XB, j)
                if mode == "gauss":
                    xs = xr + xi
                for i in outs:
                    if i < j:
                        continue
                    m = i - j
                    if m not in hc:
                        hr, hi_ = ld(HB, m)
                        hc[m] = (hr, hi_ - hr, hi_ + hr) if mode == "gauss" else (hr, hi_)
                    a = acc[i]
                    if mode == "gauss":
                        hr, hd, hs = hc[m]
                        t = (hr * xs, hd * xr, hs * xi)
                        acc[i] = t if a is None else tuple(u + v for u, v in zip(a, t))
                    elif mode == "serial":
                        hr, hi_ = hc[m]
                        if a is None:
                            acc[i] = (xr * hr - xi * hi_, xr * hi_ + xi * hr)
                        else:
                            acc[i] = ((a[0] + xr * hr) - xi * hi_, (a[1] + xr * hi_) + xi * hr)
                    else:
                        hr, hi_ = hc[m]
                        t = (xr * hr, xi * hi_, xr * hi_, xi * hr)
                        acc[i] = t if a is None else tuple(u + v for u, v in zip(a, t))
                for m in list(hc):
                    if m >= outs[-1] - j:
                        del hc[m]
            for i in outs:
                a = acc[i]
                if mode == "gauss":
                    zr, zi = a[0] - a[2], a[0] + a[1]
                elif mode == "serial":
                    zr, zi = a
                else:
                    zr, zi = a[0] - a[1], a[2] + a[3]
                wr, wi = (zr, zi) if zp is None else (zr + zp[0], zi + zp[1])
                zp = (zr, zi)
                if i % 4 == 1:
                    wr, wi = -sgn * wi, sgn * wr
                elif i % 4 == 2:
                    wr, wi = -wr, -wi
                elif i % 4 == 3:
                    wr, wi = sgn * wi, -sgn * wr
                wv = jnp.concatenate([wr, wi], axis=0).astype(jnp.bfloat16)
                A_v[pl.ds(pl.multiple_of(zs + WB + (i * NCOL + col) * 8, 8), 8), :] = pltpu.bitcast(wv, jnp.float32)
        if hi < NCH:
            A_v[pl.ds(pl.multiple_of(ZB + (hi * NCOL + col) * 16, 8), 16), :] = jnp.concatenate(zp, axis=0)

    NA = cfg["NA"]

    def conv_group(g, _):
        with scope("PH_wait_conv"):
            for cp in group_copies(g):
                cp.wait()
        with scope("PH_fwd"):
            fwd_group(g)

        @pl.when(g == NA // G - 1)
        def _():
            add_skip()
            with scope("PH_prodA"):
                def body_a(col, _):
                    prod_col(col, 0, NA, cfg["BLK_A"], "gauss")
                    return 0
                jax.lax.fori_loop(0, NCOL, body_a, 0, unroll=cfg["UNR_A"])
        return 0

    jax.lax.fori_loop(0, NG, conv_group, 0)

    with scope("PH_mod"):
        wait("z", "c")
        cf = c_v[...].astype(jnp.float32)
        sc = (cf * jax.nn.sigmoid(cf)).astype(jnp.bfloat16)
        sc = jnp.broadcast_to(sc, (16, D))
        acc = None
        for t in range(NLT):
            wait(f"wm{t}")
            part = jnp.dot(sc[:, t * 128:(t + 1) * 128], wmod_v[t * 128:(t + 1) * 128, :],
                           preferred_element_type=jnp.float32)
            acc = part if acc is None else acc + part
        md = acc[0:8, :]
        sa, ca, ga, sb, cb, gb = [md[:, j * D:(j + 1) * D] for j in range(6)]
        mod_v[0] = ga * (1.0 + ca)
        mod_v[1] = ga * sa
        mod_v[2] = 1.0 + cb
        mod_v[3] = sb
        mod_v[4] = gb

    zero = z_s[0]

    def modv(j, rows):
        v = mod_v[j]
        return jnp.concatenate([v] * (rows // 8), axis=0)

    def inverse(b, par):
        for hq in range(M // C):
            i = b * (M // C) + hq
            gm = inv_v[...]
            for lt in range(NLT):
                wsp = A_v[pl.ds(pl.multiple_of(WB + (i * NCOL + lt * 16) * 8, 8), 128), :]
                wsp = pltpu.bitcast(wsp, jnp.bfloat16)
                y_v[pl.ds(pl.multiple_of(par * M + hq * C, C), C), lt * 128:(lt + 1) * 128] = jnp.dot(
                    gm, wsp, preferred_element_type=jnp.float32)

    def pre_strip(b, par, s, chain=True):
        zz = zero if chain else 0
        ry = pl.multiple_of(par * M + s * SR, SR)
        rz = pl.multiple_of(zz + ry, SR)
        rg = pl.multiple_of(b * M + s * SR, SR)
        xf = x_v[pl.ds(rg, SR), :].astype(jnp.float32)
        gh = _ln(xf) * modv(0, SR) + modv(1, SR)
        x1 = xf + gh * y_v[pl.ds(ry, SR), :]
        y_v[pl.ds(rz, SR), :] = x1
        h2 = (_ln(x1) * modv(2, SR) + modv(3, SR)).astype(jnp.bfloat16)
        rh = pl.multiple_of(zz + 2 * M + par * (M // 2) + s * (SR // 2), 8)
        y_v[pl.ds(rh, SR // 2), :] = pltpu.bitcast(h2, jnp.float32)

    with scope("PH_pre0"):
        wait("inv", "x0")
        inverse(0, 0)
        for s in range(M // SR):
            pre_strip(0, 0, s, chain=False)

    def block(b, b0, do_pre, plo, phi, pcols, coff, pblk, pmode, first):
        par = b % 2
        npar = 1 - par
        h2 = pltpu.bitcast(y_v[pl.ds(pl.multiple_of(2 * M + par * (M // 2), 8), M // 2), :], jnp.bfloat16)
        npieces = F // TN
        cols_done = 0
        for nt in range(npieces):
            if first:
                with scope(f"PH_waitw{nt}"):
                    wait(f"wg{nt}", f"wu{nt}")
            gt = jnp.dot(h2, wg_v[:, nt * TN:(nt + 1) * TN], preferred_element_type=jnp.float32)
            up = jnp.dot(h2, wu_v[:, nt * TN:(nt + 1) * TN], preferred_element_type=jnp.float32)
            act_v[:, nt * TN:(nt + 1) * TN] = (jnp.maximum(gt, 0.0) * up).astype(jnp.bfloat16)
            while cols_done < pcols * (nt + 1) // npieces:
                col = jnp.minimum(coff + (b - b0) * pcols + cols_done, NCOL - 1)
                prod_col(col, plo, phi, pblk, pmode, zero)
                cols_done += 1
        if first:
            wait("x1")
        if do_pre:
            inverse(b + 1, npar)
        rb = pl.multiple_of(b * M, M)
        ry = pl.multiple_of(par * M, M)
        if first:
            for n, (c0, c1) in enumerate(cfg["WD_SPLIT"]):
                with scope(f"PH_waitwd{n}"):
                    wait(f"wd{c0}")
                dn = jnp.dot(act_v[...], wd_v[:, c0:c1], preferred_element_type=jnp.float32)
                if n == 0:
                    for st in range(M // SR):
                        pre_strip(b + 1, npar, st, chain=cfg["CHAIN0"])
                x1 = y_v[pl.ds(ry, M), c0:c1]
                gbv = jnp.concatenate([mod_v[4, :, c0:c1]] * (M // 8), axis=0)
                o_v[pl.ds(rb, M), c0:c1] = (x1 + gbv * dn).astype(jnp.bfloat16)
        else:
            dn = jnp.dot(act_v[...], wd_v[...], preferred_element_type=jnp.float32)
            if do_pre:
                for st in range(M // SR):
                    pre_strip(b + 1, npar, st)
            x1 = y_v[pl.ds(ry, M), :]
            o_v[pl.ds(rb, M), :] = (x1 + modv(4, M) * dn).astype(jnp.bfloat16)
        pltpu.make_async_copy(o_v.at[pl.ds(rb, M)], o_hbm.at[pl.ds(rb, M)], osem).start()

    for (b0, b1, plo, phi, pcols, coff, pblk, pmode) in cfg["FFN_PROD"]:
        with scope(f"PH_blocks{b0}"):
            if b0 == 1:
                wait("x2")
            do_pre = b1 < NB
            if b0 == 0:
                block(0, 0, do_pre, plo, phi, pcols, coff, pblk, pmode, True)
            elif b1 - b0 == 1:
                block(b0, b0, do_pre, plo, phi, pcols, coff, pblk, pmode, False)
            else:
                def body(b, _, b0=b0, do_pre=do_pre, plo=plo, phi=phi, pcols=pcols, coff=coff, pblk=pblk, pmode=pmode):
                    block(b, b0, do_pre, plo, phi, pcols, coff, pblk, pmode, False)
                    return 0
                jax.lax.fori_loop(b0, b1, body, 0)
    pltpu.make_async_copy(o_v, o_hbm, osem).wait()


def _build(cfg):
    bf = jnp.bfloat16
    hbm = pl.BlockSpec(memory_space=pl.ANY)
    scratch = [
        pltpu.VMEM((S, D), bf),
        pltpu.VMEM((S + 16, D), bf),
        pltpu.VMEM((S, D), bf),
        pltpu.VMEM((4, D), bf),
        pltpu.VMEM((NCH // cfg["G"], D, cfg["G"] * C), bf),
        pltpu.VMEM((NLT, 128), bf),
        pltpu.VMEM((D, F), bf),
        pltpu.VMEM((D, F), bf),
        pltpu.VMEM((F, D), bf),
        pltpu.VMEM((1, D), bf),
        pltpu.VMEM((D, 6 * D), bf),
        pltpu.VMEM((4, 2 * C, C), bf),
        pltpu.VMEM((C, 2 * C), bf),
        pltpu.VMEM((AROWS, 128), jnp.float32),
        pltpu.VMEM((5, 8, D), jnp.float32),
        pltpu.VMEM((3 * M, D), jnp.float32),
        pltpu.VMEM((M, F), bf),
        pltpu.VMEM((S, D), bf),
        pltpu.SMEM((8,), jnp.int32),
        pltpu.SemaphoreType.DMA((GS + 3 * NCH // cfg["G"],)),
        pltpu.SemaphoreType.DMA(()),
    ]
    return pl.pallas_call(
        functools.partial(_kernel, cfg=cfg),
        out_shape=jax.ShapeDtypeStruct((S, D), bf),
        in_specs=[hbm] * 14,
        out_specs=hbm,
        scratch_shapes=scratch,
        compiler_params=pltpu.CompilerParams(vmem_limit_bytes=110 * 1024 * 1024),
    )


@jax.jit
def pallas_adaLN_cond__ssm_conv_h3__glu_gated_reglu__prompt_kernel(
    A_q: jax.Array,
    A_k: jax.Array,
    A_v: jax.Array,
    A_shift_k: jax.Array,
    A_ssm_k: jax.Array,
    A_ssm_D: jax.Array,
    B_x: jax.Array,
    B_W_gate: jax.Array,
    B_W_up: jax.Array,
    B_W_down: jax.Array,
    c: jax.Array,
    w_mod: jax.Array,
):
    del B_x
    bf = jnp.bfloat16
    out = _build(CFG)(
        A_q.reshape(S, D), A_k.reshape(S, D), A_v.reshape(S, D), A_shift_k.T, A_ssm_k,
        A_ssm_D.reshape(NLT, 128), B_W_gate, B_W_up, B_W_down, c, w_mod,
        jnp.asarray(_FWD_NP, dtype=bf), jnp.asarray(_INV_NP, dtype=bf),
        jnp.asarray(np.array([0, 5, 3, 9, 2, 8, 1, 7], dtype=np.int32)),
    )
    return out.reshape(1, S, D)
```

```python
import functools

import numpy as np
import jax
import jax.numpy as jnp
import jax.experimental.pallas as pl
import jax.experimental.pallas.tpu as pltpu

S, D, F = 2048, 640, 1536
C = 128
NCH = S // C
NLT = D // 128
NCOL = 16 * NLT
M = 256
NB = S // M
EPS = 1e-5
GS = 32
XB = 0
HB = (NCH // 2) * NCOL * 16
WB = 2 * HB
ZB = WB + NCH * NCOL * 8
AROWS = ZB + NCH * NCOL * 16

CFG = dict(PRE0_SPLIT=((0, 3), (3, 6), (6, 8)), XB2=4, TN2=256, PRE_AFTER2=4, PRE_AFTER=4, PROD_FIRST=False, NY=4, NINV=4, CHAIN_A=True, OUT_SPLIT=((0, 256), (256, 512), (512, 640)), CHAIN0=False, WD_SPLIT=((0, 256), (256, 512), (512, 640)), UNR_A=2, SR=32, TN=256, G=2, NA=8, BLK_A=8, SCOPES=False,
           FFN_PROD=((0, 1, 8, 14, 20, 0, 1, 'serial'), (1, 3, 8, 14, 30, 20, 2, 'gauss'), (3, 7, 14, 16, 20, 0, 1, 'serial'), (7, 8, 0, 0, 0, 0, 1, 'serial')))


def _dft_consts():
    n = 2 * C
    f = np.arange(C)
    t = np.arange(C)
    th = 2 * np.pi * (f[:, None] + 0.5) * t[None, :] / n
    a = np.exp(-1j * th)
    fwd = np.stack([a.real.reshape(16, 8, C), a.imag.reshape(16, 8, C)], 1).reshape(2 * C, C)
    e = np.exp(1j * th)
    g = np.stack([e.real, -e.imag], 1).reshape(2 * C, C)
    return fwd.astype(np.float32), ((2.0 / n) * g.T).astype(np.float32)


_FWD_NP, _INV_NP = _dft_consts()


def _ln(x):
    mu = jnp.sum(x, axis=-1, keepdims=True) * (1.0 / D)
    xc = x - mu
    var = jnp.sum(xc * xc, axis=-1, keepdims=True) * (1.0 / D)
    return xc * jax.lax.rsqrt(var + EPS)


class _NoScope:
    def __enter__(self):
        return None

    def __exit__(self, *a):
        return False


def _kernel(x_hbm, k_hbm, v_hbm, sk_hbm, ssmk_hbm, ssmd_hbm, wg_hbm, wu_hbm, wd_hbm, c_hbm, wmod_hbm,
            fwd_hbm, inv_hbm, z_hbm, o_hbm,
            x_v, k_v, v_v, sk_v, ssmk_v, ssmd_v, wg_v, wu_v, wd_v, c_v, wmod_v, fwd_v, inv_v,
            A_v, B_v, mod_v, y_v, act_v, o_v, z_s, sems, osem, *, cfg):
    scope = (lambda n: jax.named_scope(n)) if cfg["SCOPES"] else (lambda n: _NoScope())
    SR, TN = cfg["SR"], cfg["TN"]
    NA = cfg["NA"]
    G = cfg["G"]
    GR = G * C
    NG = NCH // G
    copies = {}
    order = []

    def add(name, src, dst):
        cp = pltpu.make_async_copy(src, dst, sems.at[len(order)])
        copies[name] = cp
        order.append(cp)

    def group_copies(g):
        r = g * GR
        if not isinstance(g, int):
            r = pl.multiple_of(r, GR)
        return (pltpu.make_async_copy(k_hbm.at[pl.ds(r, GR)], k_v.at[pl.ds(16 + r, GR)], sems.at[GS + 3 * g]),
                pltpu.make_async_copy(v_hbm.at[pl.ds(r, GR)], v_v.at[pl.ds(r, GR)], sems.at[GS + 3 * g + 1]),
                pltpu.make_async_copy(ssmk_hbm.at[:, pl.ds(r, GR)], ssmk_v.at[g], sems.at[GS + 3 * g + 2]))

    add("z", z_hbm, z_s)
    add("sk", sk_hbm, sk_v)
    add("ssmd", ssmd_hbm, ssmd_v)
    add("fwd", fwd_hbm, fwd_v.at[0])
    for cp in order:
        cp.start()
    for g in range(NG):
        for cp in group_copies(g):
            cp.start()
    n0 = len(order)
    add("inv", inv_hbm, inv_v)
    add("c", c_hbm, c_v)
    for t in range(NLT):
        add(f"wm{t}", wmod_hbm.at[pl.ds(t * 128, 128)], wmod_v.at[pl.ds(t * 128, 128)])
    add("x0", x_hbm.at[pl.ds(0, M)], x_v.at[pl.ds(0, M)])
    for nt in range(F // TN):
        add(f"wg{nt}", wg_hbm.at[:, pl.ds(nt * TN, TN)], wg_v.at[:, pl.ds(nt * TN, TN)])
        add(f"wu{nt}", wu_hbm.at[:, pl.ds(nt * TN, TN)], wu_v.at[:, pl.ds(nt * TN, TN)])
    add("x1", x_hbm.at[pl.ds(M, M)], x_v.at[pl.ds(M, M)])
    for (c0, c1) in cfg["WD_SPLIT"]:
        add(f"wd{c0}", wd_hbm.at[:, pl.ds(c0, c1 - c0)], wd_v.at[:, pl.ds(c0, c1 - c0)])
    xb = cfg["XB2"] * M
    add("x2", x_hbm.at[pl.ds(2 * M, xb - 2 * M)], x_v.at[pl.ds(2 * M, xb - 2 * M)])
    add("x3", x_hbm.at[pl.ds(xb, S - xb)], x_v.at[pl.ds(xb, S - xb)])
    for cp in order[n0:]:
        cp.start()

    def wait(*names):
        for nm in names:
            copies[nm].wait()

    k_v[0:16, :] = jnp.zeros((16, D), jnp.bfloat16)
    wait("sk", "fwd", "ssmd", "z")
    zero = z_s[0]
    taps = sk_v[...].astype(jnp.float32)
    sgn = (1 - 2 * (jax.lax.broadcasted_iota(jnp.int32, (8, 128), 0) % 2)).astype(jnp.float32)
    f0 = fwd_v[0].astype(jnp.float32)
    f1 = []
    for fg in range(16):
        f1.append(sgn * f0[16 * fg + 8:16 * fg + 16])
        f1.append(-sgn * f0[16 * fg:16 * fg + 8])
    f1 = jnp.concatenate(f1, axis=0)
    fwd_v[1] = f1.astype(jnp.bfloat16)
    fwd_v[2] = (-f0).astype(jnp.bfloat16)
    fwd_v[3] = (-f1).astype(jnp.bfloat16)
    w = [taps[j:j + 1, :] for j in range(4)]

    def fwd_group(g, i_lo):
        for q in range(G):
            i = g * G + q
            r0 = pl.multiple_of(i * C, C)
            fm = fwd_v[i % 4]
            kf = k_v[pl.ds(r0, C + 16), :].astype(jnp.float32)
            ks = w[0] * kf[16:16 + C]
            for j in range(1, 4):
                ks = ks + w[j] * kf[16 - j:16 - j + C]
            kv = (ks * v_v[pl.ds(r0, C), :].astype(jnp.float32)).astype(jnp.bfloat16)
            xs = jnp.dot(fm, kv, preferred_element_type=jnp.float32)
            hs = jax.lax.dot_general(fm, ssmk_v[g, :, q * C:(q + 1) * C],
                                     (((1,), (1,)), ((), ())), preferred_element_type=jnp.float32)
            dst, ii = (B_v, i - NA) if i_lo > 0 else (A_v, i)
            base = pl.multiple_of(ii * (NCOL * 16), 8)
            for col in range(NCOL):
                lt, fg = divmod(col, 16)
                dst[pl.ds(base + XB + col * 16, 16), :] = xs[16 * fg:16 * fg + 16, 128 * lt:128 * lt + 128]
                dst[pl.ds(base + HB + col * 16, 16), :] = hs[16 * fg:16 * fg + 16, 128 * lt:128 * lt + 128]

    def add_skip():
        dsk = ssmd_v[...].astype(jnp.float32)
        for col in range(NCOL):
            lt = col // 16
            r = HB + col * 16
            A_v[r:r + 8, :] = A_v[r:r + 8, :] + jnp.broadcast_to(dsk[lt:lt + 1, :], (8, 128))

    def prod_col(col, lo, hi, blk, mode, zs=0):
        def ld(base, j):
            src, jj = (B_v, j - NA) if j >= NA else (A_v, j)
            v = src[pl.ds(pl.multiple_of(base + (jj * NCOL + col) * 16, 8), 16), :]
            return v[0:8], v[8:16]
        zp = None
        if lo > 0:
            zz = A_v[pl.ds(pl.multiple_of(ZB + (lo * NCOL + col) * 16, 8), 16), :]
            zp = (zz[0:8], zz[8:16])
        for i0 in range(lo, hi, blk):
            outs = list(range(i0, min(i0 + blk, hi)))
            acc = {i: None for i in outs}
            hc = {}
            for j in range(outs[-1] + 1):
                xr, xi = ld(XB, j)
                if mode == "gauss":
                    xs = xr + xi
                for i in outs:
                    if i < j:
                        continue
                    m = i - j
                    if m not in hc:
                        hr, hi_ = ld(HB, m)
                        hc[m] = (hr, hi_ - hr, hi_ + hr) if mode == "gauss" else (hr, hi_)
                    a = acc[i]
                    if mode == "gauss":
                        hr, hd, hs = hc[m]
                        t = (hr * xs, hd * xr, hs * xi)
                        acc[i] = t if a is None else tuple(u + v for u, v in zip(a, t))
                    elif mode == "serial":
                        hr, hi_ = hc[m]
                        if a is None:
                            acc[i] = (xr * hr - xi * hi_, xr * hi_ + xi * hr)
                        else:
                            acc[i] = ((a[0] + xr * hr) - xi * hi_, (a[1] + xr * hi_) + xi * hr)
                    else:
                        hr, hi_ = hc[m]
                        t = (xr * hr, xi * hi_, xr * hi_, xi * hr)
                        acc[i] = t if a is None else tuple(u + v for u, v in zip(a, t))
                for m in list(hc):
                    if m >= outs[-1] - j:
                        del hc[m]
            for i in outs:
                a = acc[i]
                if mode == "gauss":
                    zr, zi = a[0] - a[2], a[0] + a[1]
                elif mode == "serial":
                    zr, zi = a
                else:
                    zr, zi = a[0] - a[1], a[2] + a[3]
                wr, wi = (zr, zi) if zp is None else (zr + zp[0], zi + zp[1])
                zp = (zr, zi)
                if i % 4 == 1:
                    wr, wi = -sgn * wi, sgn * wr
                elif i % 4 == 2:
                    wr, wi = -wr, -wi
                elif i % 4 == 3:
                    wr, wi = sgn * wi, -sgn * wr
                wv = pltpu.pack_elementwise([wr, wi], packed_dtype=jnp.bfloat16)
                A_v[pl.ds(pl.multiple_of(zs + WB + (i * NCOL + col) * 8, 8), 8), :] = jax.lax.bitcast_convert_type(wv, jnp.float32)
        if hi < NCH:
            A_v[pl.ds(pl.multiple_of(ZB + (hi * NCOL + col) * 16, 8), 16), :] = jnp.concatenate(zp, axis=0)


    NGA = NA // G
    CA = NCOL // (NG - NGA)

    def conv_group(g, with_prod):
        with scope("PH_wait_conv"):
            for cp in group_copies(g):
                cp.wait()
        with scope("PH_fwd"):
            if with_prod and cfg["PROD_FIRST"]:
                for cc in range(CA):
                    prod_col((g - NGA) * CA + cc, 0, NA, cfg["BLK_A"], "gauss", zero if cfg["CHAIN_A"] else 0)
            fwd_group(g, NA if with_prod else 0)
            if with_prod and not cfg["PROD_FIRST"]:
                for cc in range(CA):
                    prod_col((g - NGA) * CA + cc, 0, NA, cfg["BLK_A"], "gauss", zero if cfg["CHAIN_A"] else 0)
        return 0

    jax.lax.fori_loop(0, NGA, lambda g, _: conv_group(g, False), 0)
    add_skip()
    jax.lax.fori_loop(NGA, NG, lambda g, _: conv_group(g, True), 0)

    def inverse(b):
        for hq in range(M // C):
            i = b * (M // C) + hq
            gm = inv_v[...]
            for lt in range(NLT):
                wsp = A_v[pl.ds(pl.multiple_of(WB + (i * NCOL + lt * 16) * 8, 8), 128), :]
                wsp = pltpu.bitcast(wsp, jnp.bfloat16)
                y_v[pl.ds(pl.multiple_of((b % NY) * M + hq * C, C), C), lt * 128:(lt + 1) * 128] = jnp.dot(
                    gm, wsp, preferred_element_type=jnp.float32)

    NY = cfg["NY"]
    with scope("PH_inv0"):
        wait("inv")
        for b in range(cfg["NINV"]):
            inverse(b)

    with scope("PH_mod"):
        wait("c")
        cf = c_v[...].astype(jnp.float32)
        sc = (cf * jax.nn.sigmoid(cf)).astype(jnp.bfloat16)
        sc = jnp.broadcast_to(sc, (16, D))
        acc = None
        for t in range(NLT):
            wait(f"wm{t}")
            part = jnp.dot(sc[:, t * 128:(t + 1) * 128], wmod_v[t * 128:(t + 1) * 128, :],
                           preferred_element_type=jnp.float32)
            acc = part if acc is None else acc + part
        md = acc[0:8, :]
        sa, ca, ga, sb, cb, gb = [md[:, j * D:(j + 1) * D] for j in range(6)]
        mod_v[0] = ga * (1.0 + ca)
        mod_v[1] = ga * sa
        mod_v[2] = 1.0 + cb
        mod_v[3] = sb
        mod_v[4] = gb

    def modv(j, rows):
        v = mod_v[j]
        return jnp.concatenate([v] * (rows // 8), axis=0)

    def pre_strip(b, s, chain=True):
        zz = zero if chain else 0
        par = b % 2
        ry = pl.multiple_of((b % NY) * M + s * SR, SR)
        rz = pl.multiple_of(zz + ry, SR)
        rg = pl.multiple_of(b * M + s * SR, SR)
        xf = x_v[pl.ds(rg, SR), :].astype(jnp.float32)
        gh = _ln(xf) * modv(0, SR) + modv(1, SR)
        x1 = xf + gh * y_v[pl.ds(ry, SR), :]
        y_v[pl.ds(rz, SR), :] = x1
        h2 = (_ln(x1) * modv(2, SR) + modv(3, SR)).astype(jnp.bfloat16)
        rh = pl.multiple_of(zz + NY * M + par * (M // 2) + s * (SR // 2), 8)
        y_v[pl.ds(rh, SR // 2), :] = pltpu.bitcast(h2, jnp.float32)

    with scope("PH_pre0"):
        wait("x0")
        for s in range(M // SR):
            pre_strip(0, s, chain=False)

    def block(b, b0, do_pre, plo, phi, pcols, coff, pblk, pmode, first):
        par = b % 2
        h2 = pltpu.bitcast(y_v[pl.ds(pl.multiple_of(NY * M + par * (M // 2), 8), M // 2), :], jnp.bfloat16)
        TN = cfg["TN"] if first else cfg["TN2"]
        npieces = F // TN
        cols_done = 0
        for nt in range(npieces):
            if first:
                with scope(f"PH_waitw{nt}"):
                    wait(f"wg{nt}", f"wu{nt}")
            gt = jnp.dot(h2, wg_v[:, nt * TN:(nt + 1) * TN], preferred_element_type=jnp.float32)
            up = jnp.dot(h2, wu_v[:, nt * TN:(nt + 1) * TN], preferred_element_type=jnp.float32)
            act = jnp.maximum(gt, 0.0) * up
            act_v[:, nt * TN:(nt + 1) * TN] = act.astype(jnp.bfloat16)
            if do_pre and b0 + 1 < cfg["NINV"] and nt == (cfg["PRE_AFTER"] if first else min(cfg["PRE_AFTER2"], npieces - 1)):
                y_v[pl.ds(pl.multiple_of(zero + (NY + 1) * M, 8), 8), 0:128] = act[0:8, 0:128]
            while cols_done < pcols * (nt + 1) // npieces:
                col = jnp.minimum(coff + (b - b0) * pcols + cols_done, NCOL - 1)
                prod_col(col, plo, phi, pblk, pmode, zero)
                cols_done += 1
        if first:
            wait("x1")
        if do_pre and b0 + 1 >= cfg["NINV"] and not cfg.get("NO_INV"):
            inverse(b + 1)
        rb = pl.multiple_of(b * M, M)
        ry = pl.multiple_of((b % NY) * M, M)
        if first:
            for n, (c0, c1) in enumerate(cfg["WD_SPLIT"]):
                with scope(f"PH_waitwd{n}"):
                    wait(f"wd{c0}")
                dn = jnp.dot(act_v[...], wd_v[:, c0:c1], preferred_element_type=jnp.float32)
                for st in range(*cfg["PRE0_SPLIT"][n]):
                    pre_strip(b + 1, st, chain=cfg["CHAIN0"])
                x1 = y_v[pl.ds(ry, M), c0:c1]
                gbv = jnp.concatenate([mod_v[4, :, c0:c1]] * (M // 8), axis=0)
                o_v[pl.ds(rb, M), c0:c1] = (x1 + gbv * dn).astype(jnp.bfloat16)
        elif not do_pre:
            for (c0, c1) in cfg["OUT_SPLIT"]:
                dn = jnp.dot(act_v[...], wd_v[:, c0:c1], preferred_element_type=jnp.float32)
                x1 = y_v[pl.ds(ry, M), c0:c1]
                gbv = jnp.concatenate([mod_v[4, :, c0:c1]] * (M // 8), axis=0)
                o_v[pl.ds(rb, M), c0:c1] = (x1 + gbv * dn).astype(jnp.bfloat16)
                pltpu.make_async_copy(o_v.at[pl.ds(rb, M), pl.ds(c0, c1 - c0)],
                                      o_hbm.at[pl.ds(rb, M), pl.ds(c0, c1 - c0)], osem).start()
            return
        else:
            dn = jnp.dot(act_v[...], wd_v[...], preferred_element_type=jnp.float32)
            if do_pre and not cfg.get("NO_PRE"):
                for st in range(M // SR):
                    pre_strip(b + 1, st)
            x1 = y_v[pl.ds(ry, M), :]
            o_v[pl.ds(rb, M), :] = (x1 + modv(4, M) * dn).astype(jnp.bfloat16)
        pltpu.make_async_copy(o_v.at[pl.ds(rb, M)], o_hbm.at[pl.ds(rb, M)], osem).start()

    for (b0, b1, plo, phi, pcols, coff, pblk, pmode) in cfg["FFN_PROD"]:
        with scope(f"PH_blocks{b0}"):
            if b0 == 1:
                wait("x2")
            if b0 == cfg["XB2"] - 1:
                wait("x3")
            do_pre = b1 < NB
            if b0 == 0:
                block(0, 0, do_pre, plo, phi, pcols, coff, pblk, pmode, True)
            elif b1 - b0 == 1:
                block(b0, b0, do_pre, plo, phi, pcols, coff, pblk, pmode, False)
            else:
                def body(b, _, b0=b0, do_pre=do_pre, plo=plo, phi=phi, pcols=pcols, coff=coff, pblk=pblk, pmode=pmode):
                    block(b, b0, do_pre, plo, phi, pcols, coff, pblk, pmode, False)
                    return 0
                jax.lax.fori_loop(b0, b1, body, 0)
    pltpu.make_async_copy(o_v, o_hbm, osem).wait()


def _build(cfg):
    bf = jnp.bfloat16
    hbm = pl.BlockSpec(memory_space=pl.ANY)
    scratch = [
        pltpu.VMEM((S, D), bf),
        pltpu.VMEM((S + 16, D), bf),
        pltpu.VMEM((S, D), bf),
        pltpu.VMEM((4, D), bf),
        pltpu.VMEM((NCH // cfg["G"], D, cfg["G"] * C), bf),
        pltpu.VMEM((NLT, 128), bf),
        pltpu.VMEM((D, F), bf),
        pltpu.VMEM((D, F), bf),
        pltpu.VMEM((F, D), bf),
        pltpu.VMEM((1, D), bf),
        pltpu.VMEM((D, 6 * D), bf),
        pltpu.VMEM((4, 2 * C, C), bf),
        pltpu.VMEM((C, 2 * C), bf),
        pltpu.VMEM((AROWS, 128), jnp.float32),
        pltpu.VMEM((WB, 128), jnp.float32),
        pltpu.VMEM((5, 8, D), jnp.float32),
        pltpu.VMEM(((cfg['NY'] + 1) * M + 8, D), jnp.float32),
        pltpu.VMEM((M, F), bf),
        pltpu.VMEM((S, D), bf),
        pltpu.SMEM((8,), jnp.int32),
        pltpu.SemaphoreType.DMA((GS + 3 * NCH // cfg["G"],)),
        pltpu.SemaphoreType.DMA(()),
    ]
    return pl.pallas_call(
        functools.partial(_kernel, cfg=cfg),
        out_shape=jax.ShapeDtypeStruct((S, D), bf),
        in_specs=[hbm] * 14,
        out_specs=hbm,
        scratch_shapes=scratch,
        compiler_params=pltpu.CompilerParams(vmem_limit_bytes=110 * 1024 * 1024),
    )


@jax.jit
def pallas_adaLN_cond__ssm_conv_h3__glu_gated_reglu__prompt_kernel(
    A_q: jax.Array,
    A_k: jax.Array,
    A_v: jax.Array,
    A_shift_k: jax.Array,
    A_ssm_k: jax.Array,
    A_ssm_D: jax.Array,
    B_x: jax.Array,
    B_W_gate: jax.Array,
    B_W_up: jax.Array,
    B_W_down: jax.Array,
    c: jax.Array,
    w_mod: jax.Array,
):
    del B_x
    bf = jnp.bfloat16
    out = _build(CFG)(
        A_q.reshape(S, D), A_k.reshape(S, D), A_v.reshape(S, D), A_shift_k.T, A_ssm_k,
        A_ssm_D.reshape(NLT, 128), B_W_gate, B_W_up, B_W_down, c, w_mod,
        jnp.asarray(_FWD_NP, dtype=bf), jnp.asarray(_INV_NP, dtype=bf),
        jnp.asarray(np.array([0, 5, 3, 9, 2, 8, 1, 7], dtype=np.int32)),
    )
    return out.reshape(1, S, D)
```

```python
import functools

import numpy as np
import jax
import jax.numpy as jnp
import jax.experimental.pallas as pl
import jax.experimental.pallas.tpu as pltpu

S, D, F = 2048, 640, 1536
C = 128
NCH = S // C
NLT = D // 128
NCOL = 16 * NLT
M = 256
NB = S // M
EPS = 1e-5
GS = 32


def _layout(cfg):
    xb = 0
    hb = (NCH // 2) * (NCOL * cfg["CSTR"] + cfg["JPAD"]) + cfg["HPAD"]
    wb = 2 * hb
    zb = wb + NCH * NCOL * 8
    return xb, hb, wb, zb, zb + NCH * NCOL * 16 + 8 + cfg["APAD"]


CFG = dict(BPAD=0, YPAD=8, JPAD=24, CSTR=16, HPAD=8, APAD=16, WAIT_MODE='end', PROD_POS=('stores',), PARK_A=None, H_FIRST=True, PRE0_SPLIT=((0, 3), (3, 6), (6, 8)), XB2=5, TN2=256, PRE_AFTER2=4, PRE_AFTER=4, PROD_FIRST=False, NY=2, NINV=2, CHAIN_A=True, OUT_SPLIT=((0, 256), (256, 512), (512, 640)), CHAIN0=False, WD_SPLIT=((0, 256), (256, 512), (512, 640)), UNR_A=2, SR=32, TN=256, G=2, NA=8, BLK_A=8, SCOPES=False,
           FFN_PROD=((0, 1, 8, 14, 20, 0, 1, 'serial'), (1, 4, 8, 14, 20, 20, 1, 'serial'), (4, 7, 14, 16, 27, 0, 1, 'serial'), (7, 8, 0, 0, 0, 0, 1, 'serial')))


def _dft_consts():
    n = 2 * C
    f = np.arange(C)
    t = np.arange(C)
    th = 2 * np.pi * (f[:, None] + 0.5) * t[None, :] / n
    a = np.exp(-1j * th)
    fwd = np.stack([a.real.reshape(16, 8, C), a.imag.reshape(16, 8, C)], 1).reshape(2 * C, C)
    e = np.exp(1j * th)
    g = np.stack([e.real, -e.imag], 1).reshape(2 * C, C)
    return fwd.astype(np.float32), ((2.0 / n) * g.T).astype(np.float32)


_FWD_NP, _INV_NP = _dft_consts()


def _ln(x):
    mu = jnp.sum(x, axis=-1, keepdims=True) * (1.0 / D)
    xc = x - mu
    var = jnp.sum(xc * xc, axis=-1, keepdims=True) * (1.0 / D)
    return xc * jax.lax.rsqrt(var + EPS)


class _NoScope:
    def __enter__(self):
        return None

    def __exit__(self, *a):
        return False


def _kernel(x_hbm, k_hbm, v_hbm, sk_hbm, ssmk_hbm, ssmd_hbm, wg_hbm, wu_hbm, wd_hbm, c_hbm, wmod_hbm,
            fwd_hbm, inv_hbm, z_hbm, o_hbm,
            x_v, k_v, v_v, sk_v, ssmk_v, ssmd_v, wg_v, wu_v, wd_v, c_v, wmod_v, fwd_v, inv_v,
            A_v, B_v, mod_v, y_v, act_v, o_v, dn_v, z_s, sems, osem, *, cfg):
    XB, HB, WB, ZB, AROWS = _layout(cfg)
    CS = cfg["CSTR"]
    JS = NCOL * CS + cfg["JPAD"]

    def scope(n):
        on = cfg["SCOPES"] and (cfg.get("SCOPESET") is None or any(n.startswith(p) for p in cfg["SCOPESET"]))
        return jax.named_scope(n) if on else _NoScope()
    SR, TN = cfg["SR"], cfg["TN"]
    NA = cfg["NA"]
    G = cfg["G"]
    GR = G * C
    NG = NCH // G
    copies = {}
    order = []

    def add(name, src, dst):
        cp = pltpu.make_async_copy(src, dst, sems.at[len(order)])
        copies[name] = cp
        order.append(cp)

    def group_copies(g):
        r = g * GR
        if not isinstance(g, int):
            r = pl.multiple_of(r, GR)
        return (pltpu.make_async_copy(k_hbm.at[pl.ds(r, GR)], k_v.at[pl.ds(16 + r, GR)], sems.at[GS + 3 * g]),
                pltpu.make_async_copy(v_hbm.at[pl.ds(r, GR)], v_v.at[pl.ds(r, GR)], sems.at[GS + 3 * g + 1]),
                pltpu.make_async_copy(ssmk_hbm.at[:, pl.ds(r, GR)], ssmk_v.at[g], sems.at[GS + 3 * g + 2]))

    add("z", z_hbm, z_s)
    add("sk", sk_hbm, sk_v)
    add("ssmd", ssmd_hbm, ssmd_v)
    add("fwd", fwd_hbm, fwd_v.at[0])
    for cp in order:
        cp.start()
    for g in range(NG):
        for cp in group_copies(g):
            cp.start()
    n0 = len(order)
    add("inv", inv_hbm, inv_v)
    add("c", c_hbm, c_v)
    for t in range(NLT):
        add(f"wm{t}", wmod_hbm.at[pl.ds(t * 128, 128), pl.ds(0, 5 * D)], wmod_v.at[pl.ds(t * 128, 128), pl.ds(0, 5 * D)])
    add("x0", x_hbm.at[pl.ds(0, M)], x_v.at[pl.ds(0, M)])
    for nt in range(F // TN):
        add(f"wg{nt}", wg_hbm.at[:, pl.ds(nt * TN, TN)], wg_v.at[:, pl.ds(nt * TN, TN)])
        add(f"wu{nt}", wu_hbm.at[:, pl.ds(nt * TN, TN)], wu_v.at[:, pl.ds(nt * TN, TN)])
    add("x1", x_hbm.at[pl.ds(M, M)], x_v.at[pl.ds(M, M)])
    for (c0, c1) in cfg["WD_SPLIT"]:
        add(f"wd{c0}", wd_hbm.at[:, pl.ds(c0, c1 - c0)], wd_v.at[:, pl.ds(c0, c1 - c0)])
    add("wmg", wmod_hbm.at[:, pl.ds(5 * D, D)], wmod_v.at[:, pl.ds(5 * D, D)])
    add("x2", x_hbm.at[pl.ds(2 * M, M)], x_v.at[pl.ds(2 * M, M)])
    add("x3", x_hbm.at[pl.ds(3 * M, S - 3 * M)], x_v.at[pl.ds(3 * M, S - 3 * M)])
    for cp in order[n0:]:
        cp.start()

    def wait(*names):
        for nm in names:
            copies[nm].wait()

    k_v[0:16, :] = jnp.zeros((16, D), jnp.bfloat16)
    wait("sk", "fwd", "ssmd", "z")
    zero = z_s[0]
    taps = sk_v[...].astype(jnp.float32)
    sgn = (1 - 2 * (jax.lax.broadcasted_iota(jnp.int32, (8, 128), 0) % 2)).astype(jnp.float32)
    f0 = fwd_v[0].astype(jnp.float32)
    f1 = []
    for fg in range(16):
        f1.append(sgn * f0[16 * fg + 8:16 * fg + 16])
        f1.append(-sgn * f0[16 * fg:16 * fg + 8])
    f1 = jnp.concatenate(f1, axis=0)
    fwd_v[1] = f1.astype(jnp.bfloat16)
    fwd_v[2] = (-f0).astype(jnp.bfloat16)
    fwd_v[3] = (-f1).astype(jnp.bfloat16)
    w = [taps[j:j + 1, :] for j in range(4)]

    def fwd_group(g, i_lo, mid=lambda q, where: None):
        for q in range(G):
            i = g * G + q
            r0 = pl.multiple_of(i * C, C)
            fm = fwd_v[i % 4]
            kf = k_v[pl.ds(r0, C + 16), :].astype(jnp.float32)
            ks = w[0] * kf[16:16 + C]
            for j in range(1, 4):
                ks = ks + w[j] * kf[16 - j:16 - j + C]
            kv = (ks * v_v[pl.ds(r0, C), :].astype(jnp.float32)).astype(jnp.bfloat16)
            mid(q, "shift")
            if cfg["H_FIRST"]:
                hs = jax.lax.dot_general(fm, ssmk_v[g, :, q * C:(q + 1) * C],
                                         (((1,), (1,)), ((), ())), preferred_element_type=jnp.float32)
                xs = jnp.dot(fm, kv, preferred_element_type=jnp.float32)
            else:
                xs = jnp.dot(fm, kv, preferred_element_type=jnp.float32)
                hs = jax.lax.dot_general(fm, ssmk_v[g, :, q * C:(q + 1) * C],
                                         (((1,), (1,)), ((), ())), preferred_element_type=jnp.float32)
            mid(q, "dots")
            if i_lo > 0 and q == 0 and cfg["PARK_A"]:
                A_v[pl.ds(pl.multiple_of(zero + AROWS - 8, 8), 8), :] = (hs if cfg["PARK_A"] == "h" else xs)[0:8, 0:128]
            dst, ii = (B_v, i - NA) if i_lo > 0 else (A_v, i)
            base = pl.multiple_of(ii * JS, 8)
            for col in range(NCOL):
                lt, fg = divmod(col, 16)
                dst[pl.ds(base + XB + col * CS, 16), :] = xs[16 * fg:16 * fg + 16, 128 * lt:128 * lt + 128]
                dst[pl.ds(base + HB + col * CS, 16), :] = hs[16 * fg:16 * fg + 16, 128 * lt:128 * lt + 128]
                if col % 8 == 7:
                    mid(q, f"st{col // 8}")
            mid(q, "stores")

    def add_skip():
        dsk = ssmd_v[...].astype(jnp.float32)
        for col in range(NCOL):
            lt = col // 16
            r = HB + col * CS
            A_v[r:r + 8, :] = A_v[r:r + 8, :] + jnp.broadcast_to(dsk[lt:lt + 1, :], (8, 128))

    def prod_col(col, lo, hi, blk, mode, zs=0):
        def ld(base, j):
            src, jj = (B_v, j - NA) if j >= NA else (A_v, j)
            v = src[pl.ds(pl.multiple_of(base + jj * JS + col * CS, 8), 16), :]
            return v[0:8], v[8:16]
        zp = None
        if lo > 0:
            zz = A_v[pl.ds(pl.multiple_of(ZB + (lo * NCOL + col) * 16, 8), 16), :]
            zp = (zz[0:8], zz[8:16])
        for i0 in range(lo, hi, blk):
            outs = list(range(i0, min(i0 + blk, hi)))
            acc = {i: None for i in outs}
            hc = {}
            for j in range(outs[-1] + 1):
                xr, xi = ld(XB, j)
                if mode == "gauss":
                    xs = xr + xi
                for i in outs:
                    if i < j:
                        continue
                    m = i - j
                    if m not in hc:
                        hr, hi_ = ld(HB, m)
                        hc[m] = (hr, hi_ - hr, hi_ + hr) if mode == "gauss" else (hr, hi_)
                    a = acc[i]
                    if mode == "gauss":
                        hr, hd, hs = hc[m]
                        t = (hr * xs, hd * xr, hs * xi)
                        acc[i] = t if a is None else tuple(u + v for u, v in zip(a, t))
                    elif mode == "serial":
                        hr, hi_ = hc[m]
                        if a is None:
                            acc[i] = (xr * hr - xi * hi_, xr * hi_ + xi * hr)
                        else:
                            acc[i] = ((a[0] + xr * hr) - xi * hi_, (a[1] + xr * hi_) + xi * hr)
                    else:
                        hr, hi_ = hc[m]
                        t = (xr * hr, xi * hi_, xr * hi_, xi * hr)
                        acc[i] = t if a is None else tuple(u + v for u, v in zip(a, t))
                for m in list(hc):
                    if m >= outs[-1] - j:
                        del hc[m]
            for i in outs:
                a = acc[i]
                if mode == "gauss":
                    zr, zi = a[0] - a[2], a[0] + a[1]
                elif mode == "serial":
                    zr, zi = a
                else:
                    zr, zi = a[0] - a[1], a[2] + a[3]
                wr, wi = (zr, zi) if zp is None else (zr + zp[0], zi + zp[1])
                zp = (zr, zi)
                if i % 4 == 1:
                    wr, wi = -sgn * wi, sgn * wr
                elif i % 4 == 2:
                    wr, wi = -wr, -wi
                elif i % 4 == 3:
                    wr, wi = sgn * wi, -sgn * wr
                wv = pltpu.pack_elementwise([wr, wi], packed_dtype=jnp.bfloat16)
                A_v[pl.ds(pl.multiple_of(zs + WB + (i * NCOL + col) * 8, 8), 8), :] = jax.lax.bitcast_convert_type(wv, jnp.float32)
        if hi < NCH:
            A_v[pl.ds(pl.multiple_of(ZB + (hi * NCOL + col) * 16, 8), 16), :] = jnp.concatenate(zp, axis=0)


    NGA = NA // G
    CA = NCOL // (NG - NGA)

    def wait_group(g):
        with scope("PH_wait_conv"):
            for cp in group_copies(g):
                cp.wait()

    def conv_group(g, with_prod):
        with scope("PH_fwd"):
            if not with_prod:
                fwd_group(g, 0)
            else:
                slots = [(q, wh) for q in range(G) for wh in cfg["PROD_POS"]]
                per = CA // len(slots)

                def mid(q, where):
                    if (q, where) in slots:
                        n = slots.index((q, where))
                        for cc in range(n * per, (n + 1) * per):
                            prod_col((g - NGA) * CA + cc, 0, NA, cfg["BLK_A"], "gauss", zero if cfg["CHAIN_A"] else 0)
                fwd_group(g, NA, mid)

        if cfg["WAIT_MODE"] == "end":
            @pl.when(g + 1 < NG)
            def _():
                wait_group(g + 1)
        elif cfg["WAIT_MODE"] == "all" and not with_prod:
            @pl.when(g + 1 < NGA)
            def _():
                wait_group(g + 1)
        return 0

    wait_group(0)
    jax.lax.fori_loop(0, NGA, lambda g, _: conv_group(g, False), 0)
    add_skip()
    if cfg["WAIT_MODE"] == "all":
        for g in range(NGA, NG):
            wait_group(g)
    jax.lax.fori_loop(NGA, NG, lambda g, _: conv_group(g, True), 0)

    def inverse(b):
        for hq in range(M // C):
            i = b * (M // C) + hq
            gm = inv_v[...]
            for lt in range(NLT):
                wsp = A_v[pl.ds(pl.multiple_of(WB + (i * NCOL + lt * 16) * 8, 8), 128), :]
                wsp = pltpu.bitcast(wsp, jnp.bfloat16)
                y_v[pl.ds(pl.multiple_of((b % NY) * M + hq * C, C), C), lt * 128:(lt + 1) * 128] = jnp.dot(
                    gm, wsp, preferred_element_type=jnp.float32)

    NY = cfg["NY"]
    with scope("PH_inv0"):
        wait("inv")
        for b in range(cfg["NINV"]):
            inverse(b)

    def silu_c():
        cf = c_v[...].astype(jnp.float32)
        return jnp.broadcast_to((cf * jax.nn.sigmoid(cf)).astype(jnp.bfloat16), (16, D))

    with scope("PH_mod"):
        wait("c")
        sc = silu_c()
        acc = None
        for t in range(NLT):
            wait(f"wm{t}")
            part = jnp.dot(sc[:, t * 128:(t + 1) * 128], wmod_v[t * 128:(t + 1) * 128, 0:5 * D],
                           preferred_element_type=jnp.float32)
            acc = part if acc is None else acc + part
        md = acc[0:8, :]
        sa, ca, ga, sb, cb = [md[:, j * D:(j + 1) * D] for j in range(5)]
        mod_v[0] = ga * (1.0 + ca)
        mod_v[1] = ga * sa
        mod_v[2] = 1.0 + cb
        mod_v[3] = sb

    def modv(j, rows):
        v = mod_v[j]
        return jnp.concatenate([v] * (rows // 8), axis=0)

    def pre_strip(b, s, chain=True):
        zz = zero if chain else 0
        par = b % 2
        ry = pl.multiple_of((b % NY) * M + s * SR, SR)
        rz = pl.multiple_of(zz + ry, SR)
        rg = pl.multiple_of(b * M + s * SR, SR)
        xf = x_v[pl.ds(rg, SR), :].astype(jnp.float32)
        gh = _ln(xf) * modv(0, SR) + modv(1, SR)
        x1 = xf + gh * y_v[pl.ds(ry, SR), :]
        y_v[pl.ds(rz, SR), :] = x1
        h2 = (_ln(x1) * modv(2, SR) + modv(3, SR)).astype(jnp.bfloat16)
        rh = pl.multiple_of(zz + NY * M + par * (M // 2) + s * (SR // 2), 8)
        y_v[pl.ds(rh, SR // 2), :] = pltpu.bitcast(h2, jnp.float32)

    with scope("PH_pre0"):
        wait("x0")
        for s in range(M // SR):
            pre_strip(0, s, chain=False)

    def block(b, b0, do_pre, plo, phi, pcols, coff, pblk, pmode, first):
        par = b % 2
        h2 = pltpu.bitcast(y_v[pl.ds(pl.multiple_of(NY * M + par * (M // 2), 8), M // 2), :], jnp.bfloat16)
        TN = cfg["TN"] if first else cfg["TN2"]
        npieces = F // TN
        cols_done = 0
        for nt in range(npieces):
            if first:
                with scope(f"PH_waitw{nt}"):
                    wait(f"wg{nt}", f"wu{nt}")
            gt = jnp.dot(h2, wg_v[:, nt * TN:(nt + 1) * TN], preferred_element_type=jnp.float32)
            up = jnp.dot(h2, wu_v[:, nt * TN:(nt + 1) * TN], preferred_element_type=jnp.float32)
            act = jnp.maximum(gt, 0.0) * up
            act_v[:, nt * TN:(nt + 1) * TN] = act.astype(jnp.bfloat16)
            if do_pre and b0 + 1 < cfg["NINV"] and nt == (cfg["PRE_AFTER"] if first else min(cfg["PRE_AFTER2"], npieces - 1)):
                y_v[pl.ds(pl.multiple_of(zero + (NY + 1) * M, 8), 8), 0:128] = act[0:8, 0:128]
            while cols_done < pcols * (nt + 1) // npieces:
                col = jnp.minimum(coff + (b - b0) * pcols + cols_done, NCOL - 1)
                prod_col(col, plo, phi, pblk, pmode, zero)
                cols_done += 1
        if first:
            wait("x1")
        if do_pre and b0 + 1 >= cfg["NINV"] and not cfg.get("NO_INV"):
            inverse(b + 1)
        rb = pl.multiple_of(b * M, M)
        ry = pl.multiple_of((b % NY) * M, M)
        if first:
            for n, (c0, c1) in enumerate(cfg["WD_SPLIT"]):
                with scope(f"PH_waitwd{n}"):
                    wait(f"wd{c0}")
                dn = jnp.dot(act_v[...], wd_v[:, c0:c1], preferred_element_type=jnp.float32)
                for st in range(*cfg["PRE0_SPLIT"][n]):
                    pre_strip(b + 1, st, chain=cfg["CHAIN0"])
                dn_v[:, c0:c1] = dn
            wait("wmg")
            mod_v[4] = jnp.dot(silu_c(), wmod_v[:, 5 * D:6 * D], preferred_element_type=jnp.float32)[0:8, :]
            o_v[pl.ds(rb, M), :] = (y_v[pl.ds(ry, M), :] + modv(4, M) * dn_v[...]).astype(jnp.bfloat16)
        elif not do_pre:
            for (c0, c1) in cfg["OUT_SPLIT"]:
                dn = jnp.dot(act_v[...], wd_v[:, c0:c1], preferred_element_type=jnp.float32)
                x1 = y_v[pl.ds(ry, M), c0:c1]
                gbv = jnp.concatenate([mod_v[4, :, c0:c1]] * (M // 8), axis=0)
                o_v[pl.ds(rb, M), c0:c1] = (x1 + gbv * dn).astype(jnp.bfloat16)
                pltpu.make_async_copy(o_v.at[pl.ds(rb, M), pl.ds(c0, c1 - c0)],
                                      o_hbm.at[pl.ds(rb, M), pl.ds(c0, c1 - c0)], osem).start()
            return
        else:
            dn = jnp.dot(act_v[...], wd_v[...], preferred_element_type=jnp.float32)
            if do_pre and not cfg.get("NO_PRE"):
                for st in range(M // SR):
                    pre_strip(b + 1, st)
            x1 = y_v[pl.ds(ry, M), :]
            o_v[pl.ds(rb, M), :] = (x1 + modv(4, M) * dn).astype(jnp.bfloat16)
        pltpu.make_async_copy(o_v.at[pl.ds(rb, M)], o_hbm.at[pl.ds(rb, M)], osem).start()

    for (b0, b1, plo, phi, pcols, coff, pblk, pmode) in cfg["FFN_PROD"]:
        with scope(f"PH_blocks{b0}"):
            if b0 == 1:
                wait("x2")
            do_pre = b1 < NB
            if b0 == 0:
                block(0, 0, do_pre, plo, phi, pcols, coff, pblk, pmode, True)
            elif b1 - b0 == 1:
                block(b0, b0, do_pre, plo, phi, pcols, coff, pblk, pmode, False)
            else:
                def body(b, _, b0=b0, do_pre=do_pre, plo=plo, phi=phi, pcols=pcols, coff=coff, pblk=pblk, pmode=pmode):
                    if b0 == 1:
                        pl.when(b == 2)(copies["x3"].wait)
                    block(b, b0, do_pre, plo, phi, pcols, coff, pblk, pmode, False)
                    return 0
                jax.lax.fori_loop(b0, b1, body, 0)
    pltpu.make_async_copy(o_v, o_hbm, osem).wait()


def _build(cfg):
    XB, HB, WB, ZB, AROWS = _layout(cfg)
    bf = jnp.bfloat16
    hbm = pl.BlockSpec(memory_space=pl.ANY)
    scratch = [
        pltpu.VMEM((S, D), bf),
        pltpu.VMEM((S + 16, D), bf),
        pltpu.VMEM((S, D), bf),
        pltpu.VMEM((4, D), bf),
        pltpu.VMEM((NCH // cfg["G"], D, cfg["G"] * C), bf),
        pltpu.VMEM((NLT, 128), bf),
        pltpu.VMEM((D, F), bf),
        pltpu.VMEM((D, F), bf),
        pltpu.VMEM((F, D), bf),
        pltpu.VMEM((1, D), bf),
        pltpu.VMEM((D, 6 * D), bf),
        pltpu.VMEM((4, 2 * C, C), bf),
        pltpu.VMEM((C, 2 * C), bf),
        pltpu.VMEM((AROWS, 128), jnp.float32),
        pltpu.VMEM((WB + cfg['BPAD'], 128), jnp.float32),
        pltpu.VMEM((5, 8, D), jnp.float32),
        pltpu.VMEM(((cfg['NY'] + 1) * M + 8 + cfg['YPAD'], D), jnp.float32),
        pltpu.VMEM((M, F), bf),
        pltpu.VMEM((S, D), bf),
        pltpu.VMEM((M, D), jnp.float32),
        pltpu.SMEM((8,), jnp.int32),
        pltpu.SemaphoreType.DMA((GS + 3 * NCH // cfg["G"],)),
        pltpu.SemaphoreType.DMA(()),
    ]
    return pl.pallas_call(
        functools.partial(_kernel, cfg=cfg),
        out_shape=jax.ShapeDtypeStruct((S, D), bf),
        in_specs=[hbm] * 14,
        out_specs=hbm,
        scratch_shapes=scratch,
        compiler_params=pltpu.CompilerParams(vmem_limit_bytes=110 * 1024 * 1024),
    )


@jax.jit
def pallas_adaLN_cond__ssm_conv_h3__glu_gated_reglu__prompt_kernel(
    A_q: jax.Array,
    A_k: jax.Array,
    A_v: jax.Array,
    A_shift_k: jax.Array,
    A_ssm_k: jax.Array,
    A_ssm_D: jax.Array,
    B_x: jax.Array,
    B_W_gate: jax.Array,
    B_W_up: jax.Array,
    B_W_down: jax.Array,
    c: jax.Array,
    w_mod: jax.Array,
):
    del B_x
    bf = jnp.bfloat16
    out = _build(CFG)(
        A_q.reshape(S, D), A_k.reshape(S, D), A_v.reshape(S, D), A_shift_k.T, A_ssm_k,
        A_ssm_D.reshape(NLT, 128), B_W_gate, B_W_up, B_W_down, c, w_mod,
        jnp.asarray(_FWD_NP, dtype=bf), jnp.asarray(_INV_NP, dtype=bf),
        jnp.asarray(np.array([0, 5, 3, 9, 2, 8, 1, 7], dtype=np.int32)),
    )
    return out.reshape(1, S, D)
```

```python
import numpy as np
import jax
import jax.numpy as jnp
import jax.experimental.pallas as pl
import jax.experimental.pallas.tpu as pltpu

S, D, F = 2048, 640, 1536
C = 128
NCH = S // C
NA = NCH // 2
NLT = D // 128
NCOL = 16 * NLT
G = 2
NG = NCH // G
M = 256
NB = S // M
TN = 256
SR = 32
EPS = 1e-5
GS = 32
WD_SPLIT = ((0, 256), (256, 512), (512, 640))
PRE_SPLIT = ((0, 3), (3, 6), (6, 8))
SCHEDULE = ((0, 1, 8, 14, 20, 0), (1, 4, 8, 14, 20, 20), (4, 7, 14, 16, 27, 0), (7, 8, 0, 0, 0, 0))

JS = NCOL * 16 + 24
XB = 0
HB = NA * JS + 8
WB = 2 * HB
ZB = WB + NCH * NCOL * 8
AROWS = ZB + NCH * NCOL * 16 + 24


def _dft_consts():
    n = 2 * C
    f = np.arange(C)
    t = np.arange(C)
    th = 2 * np.pi * (f[:, None] + 0.5) * t[None, :] / n
    a = np.exp(-1j * th)
    fwd = np.stack([a.real.reshape(16, 8, C), a.imag.reshape(16, 8, C)], 1).reshape(2 * C, C)
    e = np.exp(1j * th)
    g = np.stack([e.real, -e.imag], 1).reshape(2 * C, C)
    return fwd.astype(np.float32), ((2.0 / n) * g.T).astype(np.float32)


_FWD_NP, _INV_NP = _dft_consts()
_IDX_NP = np.array([0, 5, 3, 9, 2, 8, 1, 7], dtype=np.int32)


def _ln(x):
    mu = jnp.sum(x, axis=-1, keepdims=True) * (1.0 / D)
    xc = x - mu
    var = jnp.sum(xc * xc, axis=-1, keepdims=True) * (1.0 / D)
    return xc * jax.lax.rsqrt(var + EPS)


def _kernel(x_hbm, k_hbm, v_hbm, sk_hbm, ssmk_hbm, ssmd_hbm, wg_hbm, wu_hbm, wd_hbm, c_hbm, wmod_hbm,
            fwd_hbm, inv_hbm, z_hbm, o_hbm,
            x_v, k_v, v_v, sk_v, ssmk_v, ssmd_v, wg_v, wu_v, wd_v, c_v, wmod_v, fwd_v, inv_v,
            A_v, B_v, mod_v, y_v, act_v, o_v, dn_v, z_s, sems, osem):
    GR = G * C
    NGA = NA // G
    CA = NCOL // (NG - NGA)

    copies = {}
    order = []

    def add(name, src, dst):
        cp = pltpu.make_async_copy(src, dst, sems.at[len(order)])
        copies[name] = cp
        order.append(cp)

    def group_copies(g):
        r = g * GR
        if not isinstance(g, int):
            r = pl.multiple_of(r, GR)
        return (pltpu.make_async_copy(k_hbm.at[pl.ds(r, GR)], k_v.at[pl.ds(16 + r, GR)], sems.at[GS + 3 * g]),
                pltpu.make_async_copy(v_hbm.at[pl.ds(r, GR)], v_v.at[pl.ds(r, GR)], sems.at[GS + 3 * g + 1]),
                pltpu.make_async_copy(ssmk_hbm.at[:, pl.ds(r, GR)], ssmk_v.at[g], sems.at[GS + 3 * g + 2]))

    add("z", z_hbm, z_s)
    add("sk", sk_hbm, sk_v)
    add("ssmd", ssmd_hbm, ssmd_v)
    add("fwd", fwd_hbm, fwd_v.at[0])
    for cp in order:
        cp.start()
    for g in range(NG):
        for cp in group_copies(g):
            cp.start()
    n0 = len(order)
    add("inv", inv_hbm, inv_v)
    add("c", c_hbm, c_v)
    for t in range(NLT):
        add(f"wm{t}", wmod_hbm.at[pl.ds(t * 128, 128), pl.ds(0, 5 * D)], wmod_v.at[pl.ds(t * 128, 128), pl.ds(0, 5 * D)])
    add("x0", x_hbm.at[pl.ds(0, M)], x_v.at[pl.ds(0, M)])
    for nt in range(F // TN):
        add(f"wg{nt}", wg_hbm.at[:, pl.ds(nt * TN, TN)], wg_v.at[:, pl.ds(nt * TN, TN)])
        add(f"wu{nt}", wu_hbm.at[:, pl.ds(nt * TN, TN)], wu_v.at[:, pl.ds(nt * TN, TN)])
    add("x1", x_hbm.at[pl.ds(M, M)], x_v.at[pl.ds(M, M)])
    for (c0, c1) in WD_SPLIT:
        add(f"wd{c0}", wd_hbm.at[:, pl.ds(c0, c1 - c0)], wd_v.at[:, pl.ds(c0, c1 - c0)])
    add("wmg", wmod_hbm.at[:, pl.ds(5 * D, D)], wmod_v.at[:, pl.ds(5 * D, D)])
    add("x2", x_hbm.at[pl.ds(2 * M, M)], x_v.at[pl.ds(2 * M, M)])
    add("x3", x_hbm.at[pl.ds(3 * M, S - 3 * M)], x_v.at[pl.ds(3 * M, S - 3 * M)])
    assert len(order) <= GS
    for cp in order[n0:]:
        cp.start()

    def wait(*names):
        for nm in names:
            copies[nm].wait()

    k_v[0:16, :] = jnp.zeros((16, D), jnp.bfloat16)
    wait("sk", "fwd", "ssmd", "z")
    zero = z_s[0]
    taps = sk_v[...].astype(jnp.float32)
    sgn = (1 - 2 * (jax.lax.broadcasted_iota(jnp.int32, (8, 128), 0) % 2)).astype(jnp.float32)
    f0 = fwd_v[0].astype(jnp.float32)
    f1 = []
    for fg in range(16):
        f1.append(sgn * f0[16 * fg + 8:16 * fg + 16])
        f1.append(-sgn * f0[16 * fg:16 * fg + 8])
    f1 = jnp.concatenate(f1, axis=0)
    fwd_v[1] = f1.astype(jnp.bfloat16)
    fwd_v[2] = (-f0).astype(jnp.bfloat16)
    fwd_v[3] = (-f1).astype(jnp.bfloat16)
    w = [taps[j:j + 1, :] for j in range(4)]

    def fwd_group(g, second, after_chunk):
        for q in range(G):
            i = g * G + q
            r0 = pl.multiple_of(i * C, C)
            fm = fwd_v[i % 4]
            kf = k_v[pl.ds(r0, C + 16), :].astype(jnp.float32)
            ks = w[0] * kf[16:16 + C]
            for j in range(1, 4):
                ks = ks + w[j] * kf[16 - j:16 - j + C]
            kv = (ks * v_v[pl.ds(r0, C), :].astype(jnp.float32)).astype(jnp.bfloat16)
            hs = jax.lax.dot_general(fm, ssmk_v[g, :, q * C:(q + 1) * C],
                                     (((1,), (1,)), ((), ())), preferred_element_type=jnp.float32)
            xs = jnp.dot(fm, kv, preferred_element_type=jnp.float32)
            dst, ii = (B_v, i - NA) if second else (A_v, i)
            base = pl.multiple_of(ii * JS, 8)
            for col in range(NCOL):
                lt, fg = divmod(col, 16)
                dst[pl.ds(base + XB + col * 16, 16), :] = xs[16 * fg:16 * fg + 16, 128 * lt:128 * lt + 128]
                dst[pl.ds(base + HB + col * 16, 16), :] = hs[16 * fg:16 * fg + 16, 128 * lt:128 * lt + 128]
            after_chunk(q)

    def add_skip():
        dsk = ssmd_v[...].astype(jnp.float32)
        for col in range(NCOL):
            lt = col // 16
            r = HB + col * 16
            A_v[r:r + 8, :] = A_v[r:r + 8, :] + jnp.broadcast_to(dsk[lt:lt + 1, :], (8, 128))

    def prod_col(col, lo, hi, blk, gauss, zs):
        def ld(base, j):
            src, jj = (B_v, j - NA) if j >= NA else (A_v, j)
            v = src[pl.ds(pl.multiple_of(base + jj * JS + col * 16, 8), 16), :]
            return v[0:8], v[8:16]
        zp = None
        if lo > 0:
            zz = A_v[pl.ds(pl.multiple_of(ZB + (lo * NCOL + col) * 16, 8), 16), :]
            zp = (zz[0:8], zz[8:16])
        for i0 in range(lo, hi, blk):
            outs = list(range(i0, min(i0 + blk, hi)))
            acc = {i: None for i in outs}
            hc = {}
            for j in range(outs[-1] + 1):
                xr, xi = ld(XB, j)
                if gauss:
                    xs = xr + xi
                for i in outs:
                    if i < j:
                        continue
                    m = i - j
                    if m not in hc:
                        hr, hi_ = ld(HB, m)
                        hc[m] = (hr, hi_ - hr, hi_ + hr) if gauss else (hr, hi_)
                    a = acc[i]
                    if gauss:
                        hr, hd, hs = hc[m]
                        t = (hr * xs, hd * xr, hs * xi)
                        acc[i] = t if a is None else tuple(u + v for u, v in zip(a, t))
                    else:
                        hr, hi_ = hc[m]
                        if a is None:
                            acc[i] = (xr * hr - xi * hi_, xr * hi_ + xi * hr)
                        else:
                            acc[i] = ((a[0] + xr * hr) - xi * hi_, (a[1] + xr * hi_) + xi * hr)
                for m in list(hc):
                    if m >= outs[-1] - j:
                        del hc[m]
            for i in outs:
                a = acc[i]
                zr, zi = (a[0] - a[2], a[0] + a[1]) if gauss else a
                wr, wi = (zr, zi) if zp is None else (zr + zp[0], zi + zp[1])
                zp = (zr, zi)
                if i % 4 == 1:
                    wr, wi = -sgn * wi, sgn * wr
                elif i % 4 == 2:
                    wr, wi = -wr, -wi
                elif i % 4 == 3:
                    wr, wi = sgn * wi, -sgn * wr
                wv = pltpu.pack_elementwise([wr, wi], packed_dtype=jnp.bfloat16)
                A_v[pl.ds(pl.multiple_of(zs + WB + (i * NCOL + col) * 8, 8), 8), :] = (
                    jax.lax.bitcast_convert_type(wv, jnp.float32))
        if hi < NCH:
            A_v[pl.ds(pl.multiple_of(ZB + (hi * NCOL + col) * 16, 8), 16), :] = jnp.concatenate(zp, axis=0)

    def inverse(b):
        for hq in range(M // C):
            i = b * (M // C) + hq
            gm = inv_v[...]
            for lt in range(NLT):
                wsp = A_v[pl.ds(pl.multiple_of(WB + (i * NCOL + lt * 16) * 8, 8), 128), :]
                wsp = pltpu.bitcast(wsp, jnp.bfloat16)
                y_v[pl.ds(pl.multiple_of((b % 2) * M + hq * C, C), C), lt * 128:(lt + 1) * 128] = jnp.dot(
                    gm, wsp, preferred_element_type=jnp.float32)

    def wait_group(g):
        for cp in group_copies(g):
            cp.wait()

    def conv_group(g, with_prod):
        if not with_prod:
            fwd_group(g, False, lambda q: None)
        else:
            per = CA // G

            def products(q):
                for cc in range(q * per, (q + 1) * per):
                    prod_col((g - NGA) * CA + cc, 0, NA, NA, True, zero)
            fwd_group(g, True, products)

        @pl.when(g + 1 < NG)
        def _():
            wait_group(g + 1)
        return 0

    wait_group(0)
    jax.lax.fori_loop(0, NGA, lambda g, _: conv_group(g, False), 0)
    add_skip()
    jax.lax.fori_loop(NGA, NG, lambda g, _: conv_group(g, True), 0)

    wait("inv")
    inverse(0)
    inverse(1)

    def silu_c():
        cf = c_v[...].astype(jnp.float32)
        return jnp.broadcast_to((cf * jax.nn.sigmoid(cf)).astype(jnp.bfloat16), (16, D))

    wait("c")
    sc = silu_c()
    acc = None
    for t in range(NLT):
        wait(f"wm{t}")
        part = jnp.dot(sc[:, t * 128:(t + 1) * 128], wmod_v[t * 128:(t + 1) * 128, 0:5 * D],
                       preferred_element_type=jnp.float32)
        acc = part if acc is None else acc + part
    md = acc[0:8, :]
    sa, ca, ga, sb, cb = [md[:, j * D:(j + 1) * D] for j in range(5)]
    mod_v[0] = ga * (1.0 + ca)
    mod_v[1] = ga * sa
    mod_v[2] = 1.0 + cb
    mod_v[3] = sb

    def modv(j, rows):
        return jnp.concatenate([mod_v[j]] * (rows // 8), axis=0)

    def pre_strip(b, s, chain=True):
        zz = zero if chain else 0
        par = b % 2
        ry = pl.multiple_of(par * M + s * SR, SR)
        rz = pl.multiple_of(zz + ry, SR)
        rg = pl.multiple_of(b * M + s * SR, SR)
        xf = x_v[pl.ds(rg, SR), :].astype(jnp.float32)
        gh = _ln(xf) * modv(0, SR) + modv(1, SR)
        x1 = xf + gh * y_v[pl.ds(ry, SR), :]
        y_v[pl.ds(rz, SR), :] = x1
        h2 = (_ln(x1) * modv(2, SR) + modv(3, SR)).astype(jnp.bfloat16)
        rh = pl.multiple_of(zz + 2 * M + par * (M // 2) + s * (SR // 2), 8)
        y_v[pl.ds(rh, SR // 2), :] = pltpu.bitcast(h2, jnp.float32)

    wait("x0")
    for s in range(M // SR):
        pre_strip(0, s, chain=False)

    def block(b, b0, do_pre, plo, phi, pcols, coff, first):
        par = b % 2
        h2 = pltpu.bitcast(y_v[pl.ds(pl.multiple_of(2 * M + par * (M // 2), 8), M // 2), :], jnp.bfloat16)
        npieces = F // TN
        cols_done = 0
        for nt in range(npieces):
            if first:
                wait(f"wg{nt}", f"wu{nt}")
            gt = jnp.dot(h2, wg_v[:, nt * TN:(nt + 1) * TN], preferred_element_type=jnp.float32)
            up = jnp.dot(h2, wu_v[:, nt * TN:(nt + 1) * TN], preferred_element_type=jnp.float32)
            act = jnp.maximum(gt, 0.0) * up
            act_v[:, nt * TN:(nt + 1) * TN] = act.astype(jnp.bfloat16)
            if first and nt == 4:
                y_v[pl.ds(pl.multiple_of(zero + 3 * M, 8), 8), 0:128] = act[0:8, 0:128]
            while cols_done < pcols * (nt + 1) // npieces:
                col = jnp.minimum(coff + (b - b0) * pcols + cols_done, NCOL - 1)
                prod_col(col, plo, phi, 1, False, zero)
                cols_done += 1
        if first:
            wait("x1")
        if do_pre and not first:
            inverse(b + 1)
        rb = pl.multiple_of(b * M, M)
        ry = pl.multiple_of(par * M, M)
        if first:
            for n, (c0, c1) in enumerate(WD_SPLIT):
                wait(f"wd{c0}")
                dn = jnp.dot(act_v[...], wd_v[:, c0:c1], preferred_element_type=jnp.float32)
                for st in range(*PRE_SPLIT[n]):
                    pre_strip(b + 1, st, chain=False)
                dn_v[:, c0:c1] = dn
            wait("wmg")
            mod_v[4] = jnp.dot(silu_c(), wmod_v[:, 5 * D:6 * D], preferred_element_type=jnp.float32)[0:8, :]
            o_v[pl.ds(rb, M), :] = (y_v[pl.ds(ry, M), :] + modv(4, M) * dn_v[...]).astype(jnp.bfloat16)
        elif not do_pre:
            for (c0, c1) in WD_SPLIT:
                dn = jnp.dot(act_v[...], wd_v[:, c0:c1], preferred_element_type=jnp.float32)
                x1 = y_v[pl.ds(ry, M), c0:c1]
                gbv = jnp.concatenate([mod_v[4, :, c0:c1]] * (M // 8), axis=0)
                o_v[pl.ds(rb, M), c0:c1] = (x1 + gbv * dn).astype(jnp.bfloat16)
                pltpu.make_async_copy(o_v.at[pl.ds(rb, M), pl.ds(c0, c1 - c0)],
                                      o_hbm.at[pl.ds(rb, M), pl.ds(c0, c1 - c0)], osem).start()
            return
        else:
            dn = jnp.dot(act_v[...], wd_v[...], preferred_element_type=jnp.float32)
            for st in range(M // SR):
                pre_strip(b + 1, st)
            x1 = y_v[pl.ds(ry, M), :]
            o_v[pl.ds(rb, M), :] = (x1 + modv(4, M) * dn).astype(jnp.bfloat16)
        pltpu.make_async_copy(o_v.at[pl.ds(rb, M)], o_hbm.at[pl.ds(rb, M)], osem).start()

    for (b0, b1, plo, phi, pcols, coff) in SCHEDULE:
        do_pre = b1 < NB
        if b0 == 1:
            wait("x2")
        if b1 - b0 == 1:
            block(b0, b0, do_pre, plo, phi, pcols, coff, b0 == 0)
        else:
            def body(b, _, b0=b0, do_pre=do_pre, plo=plo, phi=phi, pcols=pcols, coff=coff):
                if b0 == 1:
                    pl.when(b == 2)(copies["x3"].wait)
                block(b, b0, do_pre, plo, phi, pcols, coff, False)
                return 0
            jax.lax.fori_loop(b0, b1, body, 0)
    pltpu.make_async_copy(o_v, o_hbm, osem).wait()


def _build():
    bf = jnp.bfloat16
    f32 = jnp.float32
    hbm = pl.BlockSpec(memory_space=pl.ANY)
    scratch = [
        pltpu.VMEM((S, D), bf),
        pltpu.VMEM((S + 16, D), bf),
        pltpu.VMEM((S, D), bf),
        pltpu.VMEM((4, D), bf),
        pltpu.VMEM((NG, D, G * C), bf),
        pltpu.VMEM((NLT, 128), bf),
        pltpu.VMEM((D, F), bf),
        pltpu.VMEM((D, F), bf),
        pltpu.VMEM((F, D), bf),
        pltpu.VMEM((1, D), bf),
        pltpu.VMEM((D, 6 * D), bf),
        pltpu.VMEM((4, 2 * C, C), bf),
        pltpu.VMEM((C, 2 * C), bf),
        pltpu.VMEM((AROWS, 128), f32),
        pltpu.VMEM((WB, 128), f32),
        pltpu.VMEM((5, 8, D), f32),
        pltpu.VMEM((3 * M + 16, D), f32),
        pltpu.VMEM((M, F), bf),
        pltpu.VMEM((S, D), bf),
        pltpu.VMEM((M, D), f32),
        pltpu.SMEM((8,), jnp.int32),
        pltpu.SemaphoreType.DMA((GS + 3 * NG,)),
        pltpu.SemaphoreType.DMA(()),
    ]
    return pl.pallas_call(
        _kernel,
        out_shape=jax.ShapeDtypeStruct((S, D), bf),
        in_specs=[hbm] * 14,
        out_specs=hbm,
        scratch_shapes=scratch,
        compiler_params=pltpu.CompilerParams(vmem_limit_bytes=110 * 1024 * 1024),
    )


@jax.jit
def pallas_adaLN_cond__ssm_conv_h3__glu_gated_reglu__prompt_kernel(
    A_q: jax.Array,
    A_k: jax.Array,
    A_v: jax.Array,
    A_shift_k: jax.Array,
    A_ssm_k: jax.Array,
    A_ssm_D: jax.Array,
    B_x: jax.Array,
    B_W_gate: jax.Array,
    B_W_up: jax.Array,
    B_W_down: jax.Array,
    c: jax.Array,
    w_mod: jax.Array,
):
    del B_x
    bf = jnp.bfloat16
    out = _build()(
        A_q.reshape(S, D), A_k.reshape(S, D), A_v.reshape(S, D), A_shift_k.T, A_ssm_k,
        A_ssm_D.reshape(NLT, 128), B_W_gate, B_W_up, B_W_down, c, w_mod,
        jnp.asarray(_FWD_NP, dtype=bf), jnp.asarray(_INV_NP, dtype=bf), jnp.asarray(_IDX_NP),
    )
    return out.reshape(1, S, D)
```
